```python
import os as _os
_os.environ.setdefault("JAX_PLATFORMS", "cpu")
import jax
import jax.numpy as jnp

def _softmax(x, axis=-1):
    return jax.nn.softmax(x, axis=axis)
def _gelu(x):
    return jax.nn.gelu(x, approximate=True)
def _silu(x):
    return jax.nn.silu(x)
def _sigmoid(x):
    return jax.nn.sigmoid(x)
def _layernorm(x, axis=-1, eps=1e-5):
    m = jnp.mean(x, axis=axis, keepdims=True)
    v = jnp.var(x, axis=axis, keepdims=True)
    return (x - m) / jnp.sqrt(v + eps)
def _scatter_add(tgt, idx, src, axis=0):
    return tgt.at[idx].add(src)
def _segment_sum(src, seg, n):
    return jax.ops.segment_sum(src, seg, n)
class _Rng:
    def __init__(self, key):
        self._k = key
    def _next(self):
        self._k, sub = jax.random.split(self._k)
        return sub
    def normal(self, shape):
        return jax.random.normal(self._next(), shape, dtype=jnp.bfloat16)
    def randint(self, lo, hi, shape):
        return jax.random.randint(self._next(), shape, lo, hi, dtype=jnp.int32)
    def uniform(self, shape, lo=0.0, hi=1.0):
        return jax.random.uniform(self._next(), shape, jnp.bfloat16, lo, hi)
    def permutation(self, n):
        return jax.random.permutation(self._next(), n)


kernel_name = 'gated_mix__sliding_block__sliding_local_dilated__prompt'

def setup_inputs():
    _rng = _Rng(jax.random.key(int.from_bytes(__import__("os").urandom(4), "little")))
    _w = (lambda a: (lambda t: t.astype(jnp.bfloat16) if jnp.issubdtype(t.dtype, jnp.floating) else t)(jnp.asarray(a)))
    def _A_setup():
        B, S, D = 1, 2048, 640
        return {
            "x": _w((lambda *s: _rng.normal(s) * 0.05)(B, S, D)),
            "wqkv": _w((lambda *s: _rng.normal(s) * 0.8)(D, 3 * D)),
            "wo": _w((lambda *s: _rng.normal(s) * 0.05)(D, D)),
        }
    _A_in = _A_setup()

    def _B_setup():
        B, S, D = 1, 2048, 640
        return {
            "x": _w((lambda *s: _rng.normal(s) * 0.05)(B, S, D)),
            "wqkv": _w((lambda *s: _rng.normal(s) * 0.8)(D, 3 * D)),
            "wo": _w((lambda *s: _rng.normal(s) * 0.05)(D, D)),
        }
    _B_in = _B_setup()

    return {
        "A_x": _A_in["x"],
        "A_wqkv": _A_in["wqkv"],
        "A_wo": _A_in["wo"],
        "B_x": _B_in["x"],
        "B_wqkv": _B_in["wqkv"],
        "B_wo": _B_in["wo"],
        "gate_w": _w((lambda *s: _rng.normal(s) * 0.05)(640) * 16.0),
    }

def reference(A_x, A_wqkv, A_wo, B_x, B_wqkv, B_wo, gate_w):
    def _A_ref(x, wqkv, wo):
        B, S, D = x.shape
        H = 32; Dh = D // H; W = 256
        qkv = (lambda x, *d: x.transpose(*d))((x @ wqkv).reshape(B, S, 3, H, Dh), 2, 0, 3, 1, 4)
        q, k, v = qkv[0], qkv[1], qkv[2]
        scores = jnp.einsum("bhqd,bhkd->bhqk", q, k) * (Dh ** -0.5)
        idx = jnp.arange(S)
        mask = (idx[:, None] - idx[None, :] >= 0) & (idx[:, None] - idx[None, :] < W)
        scores = jnp.where(mask[None, None], scores, -1e9)
        p = _softmax(scores, axis=-1)
        o = jnp.einsum("bhqk,bhkd->bhqd", p, v)
        return (lambda x, *d: x.transpose(*d))(o, 0, 2, 1, 3).reshape(B, S, D) @ wo

    def _B_ref(x, wqkv, wo):
        B, S, D = x.shape
        H = 32; Dh = D // H
        W, dil = 8, 2
        qkv = (lambda x, *d: x.transpose(*d))((x @ wqkv).reshape(B, S, 3, H, Dh), 2, 0, 3, 1, 4)
        q, k, v = qkv[0], qkv[1], qkv[2]
        scale = Dh ** -0.5
        pos = jnp.arange(S)
        off = jnp.arange(W) * dil
        idx = pos[:, None] - off[None, :]
        mask = idx >= 0
        idx_c = jnp.where(mask, idx, 0).reshape(-1)
        kg = k[:, :, idx_c, :].reshape(B, H, S, W, Dh)
        vg = v[:, :, idx_c, :].reshape(B, H, S, W, Dh)
        logits = jnp.einsum("bhsd,bhswd->bhsw", q, kg) * scale
        logits = jnp.where(mask[None, None, :, :], logits, -1e9)
        attn = _softmax(logits, axis=-1)
        o = jnp.einsum("bhsw,bhswd->bhsd", attn, vg)
        return (lambda x, *d: x.transpose(*d))(o, 0, 2, 1, 3).reshape(B, S, D) @ wo

    x = A_x
    g = _sigmoid((x * gate_w).sum(-1, keepdims=True))
    a = _A_ref(x, A_wqkv, A_wo)
    b = _B_ref(x, B_wqkv, B_wo)
    return g * a + (1 - g) * b
```

```python
import functools
import math

import jax
import jax.numpy as jnp
from jax import lax
from jax.experimental import pallas as pl
from jax.experimental.pallas import tpu as pltpu

S, D, H, DH = 2048, 640, 32, 20
WIN = 256
TB = 128
NB = S // TB
NT = D // 128
NG = 8
QSCALE = DH ** -0.5 * math.log2(math.e)
ONE2 = 0x3F803F80
NEG2 = 0xF149F149
R1 = 256
BPAD = 16
RB = 16
NTDIMS = (((1,), (1,)), ((), ()))

f32 = jnp.float32
bf16 = jnp.bfloat16
u32 = jnp.uint32


def _u(x):
    return pltpu.bitcast(x, u32)


def _b(x):
    return pltpu.bitcast(x, bf16)


def kernel(x_ref, wa_ref, woa_ref, wb_ref, wob_ref, gw_ref, o_ref,
           q_ref, km_ref, vt_ref, wvt_ref, wbpt_ref, wobp_ref, tmp_ref,
           kb_ref, vb_ref, ot_ref, ob_ref):
    for c in range(NT):
        cs = slice(128 * c, 128 * c + 128)
        wvt_ref[:, cs] = wa_ref[cs, 2 * D:3 * D].T
        tmp_ref[...] = wb_ref[cs, :].astype(f32).T
        for p in range(3):
            for d in range(DH):
                rows = tmp_ref[pl.ds(D * p + d, H, stride=DH), :]
                wbpt_ref[D * p + H * d:D * p + H * d + H, cs] = rows.astype(bf16)
        tmp_ref[0:D, :] = wob_ref[:, cs].astype(f32)
        for d in range(DH):
            rows = tmp_ref[pl.ds(d, H, stride=DH), :]
            wobp_ref[H * d:H * d + H, cs] = rows.astype(bf16)

    lane_p = lax.broadcasted_iota(jnp.int32, (WIN // 2, 128), 1)
    for g in range(NG):
        lg = (80 * g + 80) % 128
        km_ref[g, 0:WIN, :] = _b(jnp.where(lane_p == lg, jnp.uint32(NEG2), jnp.uint32(0)))
    vt_ref[0:2] = jnp.zeros((2, D, 128), bf16)
    kb_ref[:, 0:BPAD, :] = jnp.zeros((NT, BPAD, 128), f32)
    vb_ref[:, 0:BPAD, :] = jnp.zeros((NT, BPAD, 128), f32)

    def p1(i, carry):
        r0 = pl.multiple_of(i * R1, R1)
        xb = x_ref[pl.ds(r0, R1), :]
        qk = jnp.dot(xb, wa_ref[:, 0:2 * D], preferred_element_type=f32)
        for t in range(NT):
            q_ref[t, pl.ds(r0, R1), :] = (qk[:, 128 * t:128 * t + 128] * QSCALE).astype(bf16)
        kt = [_u(qk[:, D + 128 * t:D + 128 * t + 128].astype(bf16)) for t in range(NT)]
        lane = lax.broadcasted_iota(jnp.int32, (R1 // 2, 128), 1)
        for g in range(NG):
            t0 = (80 * g) // 128
            t1 = (80 * g + 79) // 128
            lg = (80 * g + 80) % 128
            v = jnp.where(lane == lg, jnp.uint32(0), kt[t0])
            if t1 != t0:
                v = jnp.where(lane < lg, kt[t1], v)
            km_ref[g, pl.ds(WIN + r0, R1), :] = _b(v)
        vt = lax.dot_general(wvt_ref[...], xb, NTDIMS, preferred_element_type=f32)
        for c in range(R1 // 128):
            vt_ref[2 + i * (R1 // 128) + c] = vt[:, 128 * c:128 * c + 128].astype(bf16)
        return carry

    lax.fori_loop(0, S // R1, p1, 0)

    def p2(Q, carry):
        r0 = pl.multiple_of(Q * TB, TB)
        xb = x_ref[pl.ds(r0, TB), :]
        qkvb = lax.dot_general(xb, wbpt_ref[...], NTDIMS, preferred_element_type=f32)
        for t in range(NT):
            kb_ref[t, pl.ds(BPAD + r0, TB), :] = qkvb[:, D + 128 * t:D + 128 * t + 128]
            vb_ref[t, pl.ds(BPAD + r0, TB), :] = qkvb[:, 2 * D + 128 * t:2 * D + 128 * t + 128]

        lane16 = lax.broadcasted_iota(jnp.int32, (16, 128), 1)
        grp16 = lane16 // 32
        odd = (grp16 & 1) == 1
        hi = grp16 >= 2
        row32 = lax.broadcasted_iota(jnp.int32, (32, 128), 0)
        lane32 = lax.broadcasted_iota(jnp.int32, (32, 128), 1)
        tri = row32 <= (lane32 & 31)
        row8 = lax.broadcasted_iota(jnp.int32, (8, 128), 0)
        zero16 = jnp.zeros((16, 128), u32)
        for g in range(NG):
            lg = (80 * g + 80) % 128
            bias = jnp.where(lane16 == lg, jnp.uint32(ONE2), jnp.uint32(0))
            P = []
            for r in range(4):
                q0 = pl.multiple_of(r0 + 32 * r, 32)
                ws = []
                for j in range(4):
                    f0 = DH * (4 * g + j)
                    t, lo = f0 // 128, f0 % 128
                    qt = _u(q_ref[t, pl.ds(q0, 32), :])
                    if lo + DH <= 128:
                        w = jnp.where((lane16 >= lo) & (lane16 < lo + DH), qt, bias)
                    else:
                        qt1 = _u(q_ref[t + 1, pl.ds(q0, 32), :])
                        w = jnp.where(lane16 >= lo, qt, jnp.where(lane16 < lo + DH - 128, qt1, bias))
                    ws.append(w)
                wq = _b(jnp.concatenate([ws[(gm - r) % 4] for gm in range(4)], axis=0))
                s = lax.dot_general(km_ref[g, pl.ds(q0, 288), :], wq, NTDIMS,
                                    preferred_element_type=f32)
                mrg = jnp.where(tri, s[256:288], s[0:32])
                mid = s[32:256]
                m = jnp.maximum(jnp.max(mid, axis=0, keepdims=True),
                                jnp.max(mrg, axis=0, keepdims=True))
                pmid = _u(jnp.exp2(mid - m).astype(bf16))
                pm = jnp.exp2(mrg - m)
                ptop = _u(jnp.where(tri, 0.0, pm).astype(bf16))
                pbot = _u(jnp.where(tri, pm, 0.0).astype(bf16))
                P.append([ptop] + [pmid[16 * c:16 * c + 16] for c in range(7)] + [pbot])
            T = [[] for _ in range(4)]
            for c in range(12):
                X = [P[r][c - r] if 0 <= c - r <= 8 else None for r in range(4)]
                nz = [r for r in range(4) if X[r] is not None]
                if len(nz) == 1:
                    r = nz[0]
                    for j in range(4):
                        T[j].append(jnp.where(grp16 == (j + r) % 4, X[r], zero16))
                else:
                    def sel(mask, a, b):
                        if a is None and b is None:
                            return None
                        return jnp.where(mask, zero16 if a is None else a, zero16 if b is None else b)
                    U = [sel(odd, X[(p + 1) % 4], X[p]) for p in range(4)]
                    Tp = [sel(hi, U[(p + 2) % 4], U[p]) for p in range(4)]
                    for j in range(4):
                        tj = Tp[(-j) % 4]
                        T[j].append(zero16 if tj is None else tj)
            for j in range(4):
                h = 4 * g + j
                off = (DH * h) % 16
                base = DH * h - off
                r1 = (off + DH) % 32
                acc = None
                for t in range(3):
                    v = _u(vt_ref[Q + t, base:base + 32, :])
                    halves = [v[0:8], v[8:16]]
                    hsel = (r1 // 2) // 8
                    halves[hsel] = jnp.where(row8 == (r1 // 2) % 8, jnp.uint32(ONE2), halves[hsel])
                    vw = _b(jnp.concatenate(halves, axis=0))
                    tt = _b(jnp.concatenate(T[j][4 * t:4 * t + 4], axis=0))
                    pv = jnp.dot(vw, tt, preferred_element_type=f32)
                    acc = pv if acc is None else acc + pv
                linv = 1.0 / acc[r1:r1 + 1, :]
                lo8 = (off // 8) * 8
                o = acc[lo8:lo8 + 24, :] * linv
                if j:
                    o = pltpu.roll(o, 128 - 32 * j, 1)
                ot_ref[DH * h:DH * h + DH, :] = o[off - lo8:off - lo8 + DH, :]

        for sb in range(TB // RB):
            rr = r0 + sb * RB
            qb = [qkvb[sb * RB:(sb + 1) * RB, 128 * t:128 * t + 128] * QSCALE for t in range(NT)]
            ls = []
            for w in range(8):
                acc = None
                for t in range(NT):
                    pr = qb[t] * kb_ref[t, pl.ds(BPAD + rr - 2 * w, RB), :]
                    acc = pr if acc is None else acc + pr
                acc = acc + pltpu.roll(acc, 64, 1)
                acc = acc + pltpu.roll(acc, 32, 1)
                if sb * RB < 14 and w > 0:
                    pos = rr + lax.broadcasted_iota(jnp.int32, (RB, 128), 0)
                    acc = jnp.where(pos >= 2 * w, acc, -1e30)
                ls.append(acc)
            m = functools.reduce(jnp.maximum, ls)
            ps = [jnp.exp2(l - m) for l in ls]
            linv = 1.0 / functools.reduce(lambda a, b: a + b, ps)
            for t in range(NT):
                acc = None
                for w in range(8):
                    pr = ps[w] * vb_ref[t, pl.ds(BPAD + rr - 2 * w, RB), :]
                    acc = pr if acc is None else acc + pr
                ob_ref[sb * RB:(sb + 1) * RB, 128 * t:128 * t + 128] = (acc * linv).astype(bf16)

        oa = ot_ref[...].astype(bf16).T
        a = jnp.dot(oa, woa_ref[...], preferred_element_type=f32)
        b = jnp.dot(ob_ref[...], wobp_ref[...], preferred_element_type=f32)
        z = jnp.sum(xb.astype(f32) * gw_ref[...].astype(f32), axis=-1, keepdims=True)
        gate = jax.nn.sigmoid(z)
        o_ref[pl.ds(r0, TB), :] = (b + gate * (a - b)).astype(bf16)
        return carry

    lax.fori_loop(0, NB, p2, 0)


@jax.jit
def pallas_gated_mix__sliding_block__sliding_local_dilated__prompt_kernel(A_x, A_wqkv, A_wo, B_x, B_wqkv, B_wo, gate_w):
    x = A_x.reshape(S, D)
    gw = gate_w.reshape(1, D)
    out = pl.pallas_call(
        kernel,
        out_shape=jax.ShapeDtypeStruct((S, D), bf16),
        scratch_shapes=[
            pltpu.VMEM((NT, S, 128), bf16),
            pltpu.VMEM((NG, WIN + S, 128), bf16),
            pltpu.VMEM((NB + 2, D, 128), bf16),
            pltpu.VMEM((D, D), bf16),
            pltpu.VMEM((3 * D, D), bf16),
            pltpu.VMEM((D, D), bf16),
            pltpu.VMEM((3 * D, 128), f32),
            pltpu.VMEM((NT, BPAD + S, 128), f32),
            pltpu.VMEM((NT, BPAD + S, 128), f32),
            pltpu.VMEM((D, 128), f32),
            pltpu.VMEM((TB, D), bf16),
        ],
        compiler_params=pltpu.CompilerParams(vmem_limit_bytes=100 * 1024 * 1024),
    )(x, A_wqkv, A_wo, B_wqkv, B_wo, gw)
    return out.reshape(1, S, D)
```

```python
import functools
import math

import jax
import jax.numpy as jnp
from jax import lax
from jax.experimental import pallas as pl
from jax.experimental.pallas import tpu as pltpu

S, D, H, DH = 2048, 640, 32, 20
WIN = 256
TB = 128
NB = S // TB
NT = D // 128
NG = 8
QSCALE = DH ** -0.5 * math.log2(math.e)
ONE2 = 0x3F803F80
NEG2 = 0xF149F149
HI = 0xFFFF0000
R1 = 256
HALO = 8
NTDIMS = (((1,), (1,)), ((), ()))

f32 = jnp.float32
bf16 = jnp.bfloat16
u32 = jnp.uint32


def _u(x):
    return pltpu.bitcast(x, u32)


def _b(x):
    return pltpu.bitcast(x, bf16)


def _f(x):
    return pltpu.bitcast(x, f32)


def _pack2(a, b):
    return (_u(a) >> 16) | (_u(b) & jnp.uint32(HI))


def _pack2r(a, b):
    h = jnp.uint32(0x8000)
    return ((_u(a) + h) >> 16) | ((_u(b) + h) & jnp.uint32(HI))


def _cat(xs):
    return jnp.concatenate(xs, axis=0)


def kernel(x_ref, wa_ref, woa_ref, wb_ref, wob_ref, gw_ref, o_ref,
           xm_ref, g_ref, q_ref, km_ref, vt_ref, wvt_ref, wbpt_ref, woau_ref, wobp_ref, tmp_ref,
           qb0, kb0, vb0, qb1, kb1, vb1, ot_ref, oa_ref, ob0, ob1, s0, s1, t0_, t1_, z_ref):
    sbs, tbs = (s0, s1), (t0_, t1_)
    qbs, kbs, vbs, obs = (qb0, qb1), (kb0, kb1), (vb0, vb1), (ob0, ob1)

    z_ref[0] = 0
    z_ref[1] = 0
    def deint(src, dst, doff, cs, nparts):
        for p in range(nparts):
            for e in range(DH // 2):
                rows = src[pl.ds(320 * p + e, H, stride=DH // 2), :]
                a = _cat([rows[0:8], rows[16:24]])
                b = _cat([rows[8:16], rows[24:32]])
                lo = (a & jnp.uint32(0xFFFF)) | (b << 16)
                hi = (a >> 16) | (b & jnp.uint32(HI))
                o = doff + 320 * p + 32 * e
                dst[o:o + 16, cs] = lo
                dst[o + 16:o + 32, cs] = hi

    for c in range(NT):
        cs = slice(128 * c, 128 * c + 128)
        wvt_ref[:, cs] = _u(wa_ref[cs, 2 * D:3 * D].T)
        tmp_ref[...] = _u(wb_ref[cs, :].T)
        deint(tmp_ref, wbpt_ref, 0, cs, 3)
        tmp_ref[0:D // 2, :] = _u(wob_ref[:, cs])
        deint(tmp_ref, wobp_ref, 0, cs, 1)
        woau_ref[:, cs] = _u(woa_ref[:, cs])

    lane_p = lax.broadcasted_iota(jnp.int32, (WIN // 2, 128), 1)
    for g in range(NG):
        lg = (80 * g + 80) % 128
        km_ref[g, 0:WIN // 2, :] = jnp.where(lane_p == lg, jnp.uint32(NEG2), jnp.uint32(0))
    vt_ref[0:2] = jnp.zeros((2, D // 2, 128), u32)
    kb0[:, :, 0:HALO, :] = jnp.zeros((NT, 2, HALO, 128), f32)
    vb0[:, :, 0:HALO, :] = jnp.zeros((NT, 2, HALO, 128), f32)

    def p1(i, carry):
        r0 = pl.multiple_of(i * R1, R1)
        h0 = pl.multiple_of(i * (R1 // 2), R1 // 2)
        xb = x_ref[pl.ds(r0, R1), :]
        qk = jnp.dot(xb, wa_ref[:, 0:2 * D], preferred_element_type=f32)
        for t in range(NT):
            q_ref[t, pl.ds(h0, R1 // 2), :] = _u((qk[:, 128 * t:128 * t + 128] * QSCALE).astype(bf16))
        kt = [_u(qk[:, D + 128 * t:D + 128 * t + 128].astype(bf16)) for t in range(NT)]
        lane = lax.broadcasted_iota(jnp.int32, (R1 // 2, 128), 1)
        for g in range(NG):
            t0 = (80 * g) // 128
            t1 = (80 * g + 79) // 128
            lg = (80 * g + 80) % 128
            v = jnp.where(lane == lg, jnp.uint32(0), kt[t0])
            if t1 != t0:
                v = jnp.where(lane < lg, kt[t1], v)
            km_ref[g, pl.ds(WIN // 2 + h0, R1 // 2), :] = v
        xf = xb.astype(f32)
        xp = _cat([_pack2(xf[16 * k:16 * k + 8], xf[16 * k + 8:16 * k + 16]) for k in range(R1 // 16)])
        vt = lax.dot_general(_b(wvt_ref[...]), _b(xp), NTDIMS, preferred_element_type=f32)
        for c in range(R1 // 128):
            vt_ref[2 + i * (R1 // 128) + c] = _u(vt[:, 128 * c:128 * c + 128].astype(bf16))
        xw = _u(xb)
        ev = _f(xw << 16)
        od = _f(xw & jnp.uint32(HI))
        xm = _cat([z[8 * k:8 * k + 8] for k in range(R1 // 16) for z in (ev, od)])
        xm_ref[pl.ds(h0, R1 // 2), :] = _u(xm.astype(bf16))
        z = jnp.sum(xf * gw_ref[...].astype(f32), axis=-1, keepdims=True)
        g_ref[pl.ds(r0, R1), :] = jnp.broadcast_to(jax.nn.sigmoid(z), (R1, 128))
        return carry

    lax.fori_loop(0, S // R1, p1, 0)

    def mo(v, m):
        return v if isinstance(v, int) else pl.multiple_of(v, m)

    def pb_unit(Qn, pn, n):
        h0 = mo(Qn * (TB // 2), TB // 2)
        xb = _b(xm_ref[pl.ds(h0, TB // 2), :])
        w = _b(wbpt_ref[64 * n:64 * n + 64, :])
        res = lax.dot_general(xb, w, NTDIMS, preferred_element_type=f32)
        p, t = n // NT, n % NT
        if p == 0:
            qbs[pn][t] = res * QSCALE
        else:
            dst = (kbs if p == 1 else vbs)[pn]
            for k in range(TB // 16):
                for e in range(2):
                    dst[t, e, HALO + 8 * k:HALO + 8 * k + 8, :] = res[16 * k + 8 * e:16 * k + 8 * e + 8]

    def halo_copy(par):
        for bufs in (kbs, vbs):
            bufs[par][:, :, 0:HALO, :] = bufs[1 - par][:, :, TB // 2:TB // 2 + HALO, :]

    def oa_transpose():
        for t in range(NT):
            oa_ref[:, 128 * t:128 * t + 128] = _u(ot_ref[128 * t:128 * t + 128, :].astype(bf16).T)

    def out_b(po, n):
        return jnp.dot(_b(obs[po][...]), _b(wobp_ref[:, 128 * n:128 * n + 128]), preferred_element_type=f32)

    def out_a(Qo, n, b):
        a = jnp.dot(_b(oa_ref[...]), _b(woau_ref[:, 128 * n:128 * n + 128]), preferred_element_type=f32)
        r0 = mo(Qo * TB, TB)
        gate = g_ref[pl.ds(r0, TB), :]
        o_ref[pl.ds(r0, TB), 128 * n:128 * n + 128] = (b + gate * (a - b)).astype(bf16)

    def battn(par, first):
        qb, kb, vb, ob = qbs[par], kbs[par], vbs[par], obs[par]
        for i in range(TB // 16):
            q = [qb[t, 16 * i:16 * i + 16, :] for t in range(NT)]

            def win(buf, t, w):
                o = HALO + 8 * i - w
                return _cat([buf[t, 0, o:o + 8, :], buf[t, 1, o:o + 8, :]])
            ls = []
            for w in range(8):
                acc = None
                for t in range(NT):
                    pr = q[t] * win(kb, t, w)
                    acc = pr if acc is None else acc + pr
                acc = acc + pltpu.roll(acc, 64, 1)
                acc = acc + pltpu.roll(acc, 32, 1)
                if first and i == 0 and w > 0:
                    pos = lax.broadcasted_iota(jnp.int32, (16, 128), 0) & 7
                    acc = jnp.where(pos >= w, acc, -1e30)
                ls.append(acc)
            m = functools.reduce(jnp.maximum, ls)
            ps = [jnp.exp2(l - m) for l in ls]
            linv = 1.0 / functools.reduce(lambda a, b: a + b, ps)
            for t in range(NT):
                acc = None
                for w in range(8):
                    pr = ps[w] * win(vb, t, w)
                    acc = pr if acc is None else acc + pr
                acc = acc * linv
                ob[8 * i:8 * i + 8, 128 * t:128 * t + 128] = _pack2r(acc[0:8], acc[8:16])

    def attn_consts():
        lane16 = lax.broadcasted_iota(jnp.int32, (16, 128), 1)
        grp16 = lane16 // 32
        row32 = lax.broadcasted_iota(jnp.int32, (32, 128), 0)
        lane32 = lax.broadcasted_iota(jnp.int32, (32, 128), 1)
        tri = row32 <= (lane32 & 31)
        ones = jnp.full((32, 128), -1, jnp.int32)
        tb = _f(jnp.where(tri, ones, 0))
        mbot = _cat([_pack2(tb[0:8], tb[8:16]), _pack2(tb[16:24], tb[24:32])])
        return dict(za=z_ref[0], zb=z_ref[1], lane16=lane16, grp16=grp16, odd=(grp16 & 1) == 1, hi=grp16 >= 2, tri=tri,
                    mbot=mbot, mtop=~mbot,
                    row8=lax.broadcasted_iota(jnp.int32, (8, 128), 0),
                    zero16=jnp.zeros((16, 128), u32))

    def qk(Q, g, C):
        lane16 = C["lane16"]
        lg = (80 * g + 80) % 128
        bias = jnp.where(lane16 == lg, jnp.uint32(ONE2), jnp.uint32(0))
        ss = []
        for r in range(4):
            q0 = mo(Q * (TB // 2) + 16 * r, 16)
            ws = []
            for j in range(4):
                f0 = DH * (4 * g + j)
                t, lo = f0 // 128, f0 % 128
                qt = q_ref[t, pl.ds(q0, 16), :]
                if lo + DH <= 128:
                    w = jnp.where((lane16 >= lo) & (lane16 < lo + DH), qt, bias)
                else:
                    qt1 = q_ref[t + 1, pl.ds(q0, 16), :]
                    w = jnp.where(lane16 >= lo, qt, jnp.where(lane16 < lo + DH - 128, qt1, bias))
                ws.append(w)
            wq = _b(_cat([ws[(gm - r) % 4] for gm in range(4)]))
            s = lax.dot_general(_b(km_ref[g, pl.ds(q0, 144), :]), wq, NTDIMS,
                                preferred_element_type=f32)
            mrg = jnp.where(C["tri"], s[256:288], s[0:32])
            mid = s[32:256]
            sbs[g % 2][r + C['za'], 0:224, :] = mid
            sbs[g % 2][r + C['za'], 224:256, :] = mrg
            ss.append(jnp.maximum(jnp.max(mid, axis=0, keepdims=True),
                                  jnp.max(mrg, axis=0, keepdims=True)))
        return ss

    def softmax(g, ms, C):
        zero16 = C["zero16"]
        sb, tb = sbs[g % 2], tbs[g % 2]

        def chunk(r, k):
            p = jnp.exp2(sb[r + C['zb'], 32 * k:32 * k + 32, :] - ms[r])
            return _cat([_pack2(p[0:8], p[8:16]), _pack2(p[16:24], p[24:32])])
        pw = [None] * 4
        for c in range(12):
            X = [None] * 4
            for r in range(4):
                k = c - r
                if k == 0:
                    pw[r] = chunk(r, 7)
                    X[r] = pw[r] & C["mtop"]
                elif k == 8:
                    X[r] = pw[r] & C["mbot"]
                elif 0 < k < 8:
                    X[r] = chunk(r, k - 1)
            nz = [r for r in range(4) if X[r] is not None]
            if len(nz) == 1:
                r = nz[0]
                T = [jnp.where(C["grp16"] == (j + r) % 4, X[r], zero16) for j in range(4)]
            else:
                def sel(mask, a, b):
                    if a is None and b is None:
                        return None
                    return jnp.where(mask, zero16 if a is None else a, zero16 if b is None else b)
                U = [sel(C["odd"], X[(p + 1) % 4], X[p]) for p in range(4)]
                Tp = [sel(C["hi"], U[(p + 2) % 4], U[p]) for p in range(4)]
                T = [zero16 if Tp[(-j) % 4] is None else Tp[(-j) % 4] for j in range(4)]
            for j in range(4):
                tb[j + C['za'], 16 * c:16 * c + 16, :] = T[j]

    def pv(Q, g, T, C):
        for j in range(4):
            h = 4 * g + j
            off = (DH * h) % 16
            base = DH * h - off
            r1 = (off + DH) % 32
            acc = None
            for t in range(3):
                v = vt_ref[Q + t, base // 2:base // 2 + 16, :]
                halves = [v[0:8], v[8:16]]
                hsel = (r1 // 2) // 8
                halves[hsel] = jnp.where(C["row8"] == (r1 // 2) % 8, jnp.uint32(ONE2), halves[hsel])
                vw = _b(_cat(halves))
                tt = _b(tbs[g % 2][j + C['zb'], 64 * t:64 * t + 64, :])
                d = jnp.dot(vw, tt, preferred_element_type=f32)
                acc = d if acc is None else acc + d
            linv = 1.0 / acc[r1:r1 + 1, :]
            lo8 = (off // 8) * 8
            o = acc[lo8:lo8 + 24, :] * linv
            if j:
                o = pltpu.roll(o, 128 - 32 * j, 1)
            ot_ref[DH * h:DH * h + DH, :] = o[off - lo8:off - lo8 + DH, :]

    def block(Q, par, mode):
        C = attn_consts()
        bstate = {}

        def U_pb(Qn, pn, n):
            return lambda: pb_unit(Qn, pn, n)

        def U_b(po, n):
            def f():
                bstate[n] = out_b(po, n)
            return f

        def U_a(Qo, n):
            return lambda: out_a(Qo, n, bstate.pop(n))

        if mode == "first":
            pbs = [U_pb(Q, par, n) for n in range(15)] + [U_pb(Q + 1, 1 - par, n) for n in range(15)]
            slots = [pbs[0:1], pbs[1:5], pbs[5:8], pbs[8:11], pbs[11:15], pbs[15:18], pbs[18:21],
                     pbs[21:24], pbs[24:28], pbs[28:30]]
        else:
            halo_copy(par)
            oa_transpose()
            battn(par, False)
            o = []
            for n in range(NT):
                o += [U_b(1 - par, n), U_a(Q - 1, n)]
            if mode == "mid":
                pbs = [U_pb(Q + 1, 1 - par, n) for n in range(15)]
                slots = [pbs[0:1], pbs[1:4],
                         [o[0], pbs[4], o[1]], [o[2], pbs[5]], [o[3], pbs[6], pbs[7]], [o[4], pbs[8]],
                         [o[5], pbs[9], pbs[10]], [o[6], pbs[11]],
                         [o[7], pbs[12], pbs[13], o[8]], [o[9], pbs[14]]]
            else:
                slots = [[], o[0:2], o[2:3], o[3:4], o[4:5], o[5:6], o[6:7], o[7:8], o[8:10], []]

        def run(us):
            for u in us:
                u()

        run(slots[0])
        ss = qk(Q, 0, C)
        run(slots[1])
        for g in range(NG):
            T = softmax(g, ss, C)
            if g + 1 < NG:
                ss = qk(Q, g + 1, C)
            else:
                pass
            if g + 1 < NG:
                pv(Q, g, T, C)
                run(slots[2 + g])
            else:
                pv(Q, g, T, C)
                run(slots[2 + g])
            if mode == "first" and g == 3:
                battn(par, True)
        if mode == "last":
            bs = [out_b(par, n) for n in range(NT)]
            oa_transpose()
            for n in range(NT):
                out_a(Q, n, bs[n])

    block(0, 0, "first")

    def p2(i, carry):
        block(2 * i + 1, 1, "mid")
        block(2 * i + 2, 0, "mid")
        return carry

    lax.fori_loop(0, (NB - 2) // 2, p2, 0)
    block(NB - 1, 1, "last")


@jax.jit
def pallas_gated_mix__sliding_block__sliding_local_dilated__prompt_kernel(A_x, A_wqkv, A_wo, B_x, B_wqkv, B_wo, gate_w):
    x = A_x.reshape(S, D)
    gw = gate_w.reshape(1, D)
    bbuf = [pltpu.VMEM((NT, TB, 128), f32), pltpu.VMEM((NT, 2, HALO + TB // 2, 128), f32),
            pltpu.VMEM((NT, 2, HALO + TB // 2, 128), f32)]
    out = pl.pallas_call(
        kernel,
        out_shape=jax.ShapeDtypeStruct((S, D), bf16),
        scratch_shapes=[
            pltpu.VMEM((S // 2, D), u32),
            pltpu.VMEM((S, 128), f32),
            pltpu.VMEM((NT, S // 2, 128), u32),
            pltpu.VMEM((NG, (WIN + S) // 2, 128), u32),
            pltpu.VMEM((NB + 2, D // 2, 128), u32),
            pltpu.VMEM((D // 2, D), u32),
            pltpu.VMEM((3 * D // 2, D), u32),
            pltpu.VMEM((D // 2, D), u32),
            pltpu.VMEM((D // 2, D), u32),
            pltpu.VMEM((3 * D // 2, 128), u32),
        ] + bbuf + bbuf + [
            pltpu.VMEM((D, 128), f32),
            pltpu.VMEM((TB // 2, D), u32),
            pltpu.VMEM((TB // 2, D), u32),
            pltpu.VMEM((TB // 2, D), u32),
            pltpu.VMEM((4, 256, 128), f32),
            pltpu.VMEM((4, 256, 128), f32),
            pltpu.VMEM((4, 192, 128), u32),
            pltpu.VMEM((4, 192, 128), u32),
            pltpu.SMEM((2,), jnp.int32),
        ],
        compiler_params=pltpu.CompilerParams(vmem_limit_bytes=100 * 1024 * 1024),
    )(x, A_wqkv, A_wo, B_wqkv, B_wo, gw)
    return out.reshape(1, S, D)
```

```python
import functools
import math

import jax
import jax.numpy as jnp
from jax import lax
from jax.experimental import pallas as pl
from jax.experimental.pallas import tpu as pltpu

S, D, H, DH = 2048, 640, 32, 20
WIN = 256
TB = 128
NB = S // TB
NT = D // 128
NG = 8
QSCALE = DH ** -0.5 * math.log2(math.e)
ONE2 = 0x3F803F80
NEG2 = 0xF149F149
HI = 0xFFFF0000
R1 = 256
R2 = 512
HALO = 8
NTDIMS = (((1,), (1,)), ((), ()))

f32 = jnp.float32
bf16 = jnp.bfloat16
u32 = jnp.uint32


def _u(x):
    return pltpu.bitcast(x, u32)


def _b(x):
    return pltpu.bitcast(x, bf16)


def _f(x):
    return pltpu.bitcast(x, f32)


def _pack2(a, b):
    return (_u(a) >> 16) | (_u(b) & jnp.uint32(HI))


def _pack2r(a, b):
    h = jnp.uint32(0x8000)
    return ((_u(a) + h) >> 16) | ((_u(b) + h) & jnp.uint32(HI))


def _cat(xs):
    return jnp.concatenate(xs, axis=0)


def kernel(x_hbm, wa_hbm, woa_hbm, wb_hbm, wob_hbm, gw_hbm, o_hbm,
           x_ref, wa_ref, woa_ref, wb_ref, wob_ref, gw_ref, o_ref, sem_in, sem_x, sem_wb, sem_o,
           xm_ref, g_ref, q_ref, km_ref, vt_ref, wvt_ref, wbpt_ref, woau_ref, wobp_ref, tmp_ref,
           qb0, kb0, vb0, qb1, kb1, vb1, ot_ref, oa_ref, ob0, ob1, s0, s1, t0_, t1_, z_ref):
    sbs, tbs = (s0, s1), (t0_, t1_)
    qbs, kbs, vbs, obs = (qb0, qb1), (kb0, kb1), (vb0, vb1), (ob0, ob1)

    def mo(v, m):
        return v if isinstance(v, int) else pl.multiple_of(v, m)

    def cp_x(r0, n, sem):
        return pltpu.make_async_copy(x_hbm.at[pl.ds(r0, n), :], x_ref.at[pl.ds(r0, n), :], sem)

    def cp_xl(p):
        return cp_x(mo(R2 * (p + 1), R2), R2, sem_x.at[p])

    def cp_wa(p):
        return pltpu.make_async_copy(wa_hbm.at[:, pl.ds(D * p, D)], wa_ref.at[p], sem_in.at[p])

    def cp_wb(p):
        return pltpu.make_async_copy(wb_hbm.at[:, pl.ds(mo(D * p, 128), D)], wb_ref.at[p], sem_wb.at[p])

    def cp_o(r0, n, k):
        return pltpu.make_async_copy(o_ref.at[pl.ds(r0, n), :], o_hbm.at[pl.ds(r0, n), :], sem_o.at[k])

    c_x0, c_x1 = cp_x(0, R1, sem_in.at[3]), cp_x(R1, R1, sem_in.at[4])
    c_gw = pltpu.make_async_copy(gw_hbm, gw_ref, sem_in.at[5])
    c_woa = pltpu.make_async_copy(woa_hbm, woa_ref, sem_in.at[6])
    c_wob = pltpu.make_async_copy(wob_hbm, wob_ref, sem_in.at[7])
    for c in (c_x0, cp_wa(0), c_gw, c_x1, cp_wa(2), cp_wa(1), cp_xl(0), cp_wb(0), cp_xl(1), cp_wb(1), cp_xl(2),
              cp_wb(2), c_woa, c_wob):
        c.start()

    z_ref[0] = 0
    z_ref[1] = 0

    def deint(src, dst, doff, cs):
        for e in range(DH // 2):
            rows = src[pl.ds(e, H, stride=DH // 2), :]
            a = _cat([rows[0:8], rows[16:24]])
            b = _cat([rows[8:16], rows[24:32]])
            lo = (a & jnp.uint32(0xFFFF)) | (b << 16)
            hi = (a >> 16) | (b & jnp.uint32(HI))
            dst[pl.ds(mo(doff + 32 * e, 16), 16), cs] = lo
            dst[pl.ds(mo(doff + 32 * e + 16, 16), 16), cs] = hi

    lane_p = lax.broadcasted_iota(jnp.int32, (WIN // 2, 128), 1)
    for g in range(NG):
        lg = (80 * g + 80) % 128
        km_ref[g, 0:WIN // 2, :] = jnp.where(lane_p == lg, jnp.uint32(NEG2), jnp.uint32(0))
    vt_ref[0:2] = jnp.zeros((2, D // 2, 128), u32)
    kb0[:, :, 0:HALO, :] = jnp.zeros((NT, 2, HALO, 128), f32)
    vb0[:, :, 0:HALO, :] = jnp.zeros((NT, 2, HALO, 128), f32)

    def p1_q(i):
        r0, h0 = mo(i * R1, R1), mo(i * (R1 // 2), R1 // 2)
        xb = x_ref[pl.ds(r0, R1), :]
        q = jnp.dot(xb, wa_ref[0], preferred_element_type=f32)
        for t in range(NT):
            q_ref[t, pl.ds(h0, R1 // 2), :] = _u((q[:, 128 * t:128 * t + 128] * QSCALE).astype(bf16))
        xw = _u(xb)
        ev = _f(xw << 16)
        od = _f(xw & jnp.uint32(HI))
        xm = _cat([z[8 * k:8 * k + 8] for k in range(R1 // 16) for z in (ev, od)])
        xm_ref[pl.ds(h0, R1 // 2), :] = _u(xm.astype(bf16))
        z = jnp.sum(xb.astype(f32) * gw_ref[...].astype(f32), axis=-1, keepdims=True)
        g_ref[pl.ds(r0, R1), :] = jnp.broadcast_to(jax.nn.sigmoid(z), (R1, 128))

    def p1_k(i):
        r0, h0 = mo(i * R1, R1), mo(i * (R1 // 2), R1 // 2)
        xb = x_ref[pl.ds(r0, R1), :]
        k = jnp.dot(xb, wa_ref[1], preferred_element_type=f32)
        kt = [_u(k[:, 128 * t:128 * t + 128].astype(bf16)) for t in range(NT)]
        lane = lax.broadcasted_iota(jnp.int32, (R1 // 2, 128), 1)
        for g in range(NG):
            t0 = (80 * g) // 128
            t1 = (80 * g + 79) // 128
            lg = (80 * g + 80) % 128
            v = jnp.where(lane == lg, jnp.uint32(0), kt[t0])
            if t1 != t0:
                v = jnp.where(lane < lg, kt[t1], v)
            km_ref[g, pl.ds(WIN // 2 + h0, R1 // 2), :] = v

    def p1_v(i):
        r0 = mo(i * R1, R1)
        xf = x_ref[pl.ds(r0, R1), :].astype(f32)
        xp = _cat([_pack2(xf[16 * k:16 * k + 8], xf[16 * k + 8:16 * k + 16]) for k in range(R1 // 16)])
        vt = lax.dot_general(_b(wvt_ref[...]), _b(xp), NTDIMS, preferred_element_type=f32)
        for c in range(R1 // 128):
            vt_ref[2 + i * (R1 // 128) + c] = _u(vt[:, 128 * c:128 * c + 128].astype(bf16))

    c_x0.wait()
    cp_wa(0).wait()
    c_gw.wait()
    p1_q(0)
    c_x1.wait()
    p1_q(1)
    cp_wa(2).wait()
    cp_wa(1).wait()
    for c in range(NT):
        cs = slice(128 * c, 128 * c + 128)
        wvt_ref[:, cs] = _u(wa_ref[2, cs, :].T)
    p1_k(0)
    p1_k(1)
    p1_v(0)
    p1_v(1)

    def p1(p, carry):
        cp_xl(p).wait()
        cp_wb(p).wait()
        for c in range(NT):
            cs = slice(128 * c, 128 * c + 128)
            tmp_ref[c] = _u(wb_ref[p, cs, :].T)
            deint(tmp_ref.at[c], wbpt_ref, 320 * p, cs)
        for i in (2 * p + 2, 2 * p + 3):
            p1_q(i)
            p1_k(i)
            p1_v(i)
        return carry

    lax.fori_loop(0, 3, p1, 0)

    c_woa.wait()
    c_wob.wait()
    for c in range(NT):
        cs = slice(128 * c, 128 * c + 128)
        tmp_ref[c] = _u(wob_ref[:, cs])
        deint(tmp_ref.at[c], wobp_ref, 0, cs)
        woau_ref[:, cs] = _u(woa_ref[:, cs])

    def pb_unit(Qn, pn, n):
        h0 = mo(Qn * (TB // 2), TB // 2)
        xb = _b(xm_ref[pl.ds(h0, TB // 2), :])
        w = _b(wbpt_ref[64 * n:64 * n + 64, :])
        res = lax.dot_general(xb, w, NTDIMS, preferred_element_type=f32)
        p, t = n // NT, n % NT
        if p == 0:
            qbs[pn][t] = res * QSCALE
        else:
            dst = (kbs if p == 1 else vbs)[pn]
            for k in range(TB // 16):
                for e in range(2):
                    dst[t, e, HALO + 8 * k:HALO + 8 * k + 8, :] = res[16 * k + 8 * e:16 * k + 8 * e + 8]

    def halo_copy(par):
        for bufs in (kbs, vbs):
            bufs[par][:, :, 0:HALO, :] = bufs[1 - par][:, :, TB // 2:TB // 2 + HALO, :]

    def oa_transpose():
        for t in range(NT):
            oa_ref[:, 128 * t:128 * t + 128] = _u(ot_ref[128 * t:128 * t + 128, :].astype(bf16).T)

    def out_b(po, n):
        return jnp.dot(_b(obs[po][...]), _b(wobp_ref[:, 128 * n:128 * n + 128]), preferred_element_type=f32)

    def out_a(Qo, n, b):
        a = jnp.dot(_b(oa_ref[...]), _b(woau_ref[:, 128 * n:128 * n + 128]), preferred_element_type=f32)
        r0 = mo(Qo * TB, TB)
        gate = g_ref[pl.ds(r0, TB), :]
        o_ref[pl.ds(r0, TB), 128 * n:128 * n + 128] = (b + gate * (a - b)).astype(bf16)

    def battn(par, first):
        qb, kb, vb, ob = qbs[par], kbs[par], vbs[par], obs[par]
        for i in range(TB // 16):
            q = [qb[t, 16 * i:16 * i + 16, :] for t in range(NT)]

            def win(buf, t, w):
                o = HALO + 8 * i - w
                return _cat([buf[t, 0, o:o + 8, :], buf[t, 1, o:o + 8, :]])
            ls = []
            for w in range(8):
                acc = None
                for t in range(NT):
                    pr = q[t] * win(kb, t, w)
                    acc = pr if acc is None else acc + pr
                acc = acc + pltpu.roll(acc, 64, 1)
                acc = acc + pltpu.roll(acc, 32, 1)
                if first and i == 0 and w > 0:
                    pos = lax.broadcasted_iota(jnp.int32, (16, 128), 0) & 7
                    acc = jnp.where(pos >= w, acc, -1e30)
                ls.append(acc)
            m = functools.reduce(jnp.maximum, ls)
            ps = [jnp.exp2(l - m) for l in ls]
            linv = 1.0 / functools.reduce(lambda a, b: a + b, ps)
            for t in range(NT):
                acc = None
                for w in range(8):
                    pr = ps[w] * win(vb, t, w)
                    acc = pr if acc is None else acc + pr
                acc = acc * linv
                ob[8 * i:8 * i + 8, 128 * t:128 * t + 128] = _pack2r(acc[0:8], acc[8:16])

    def attn_consts():
        lane16 = lax.broadcasted_iota(jnp.int32, (16, 128), 1)
        grp16 = lane16 // 32
        row32 = lax.broadcasted_iota(jnp.int32, (32, 128), 0)
        lane32 = lax.broadcasted_iota(jnp.int32, (32, 128), 1)
        tri = row32 <= (lane32 & 31)
        ones = jnp.full((32, 128), -1, jnp.int32)
        tb = _f(jnp.where(tri, ones, 0))
        mbot = _cat([_pack2(tb[0:8], tb[8:16]), _pack2(tb[16:24], tb[24:32])])
        return dict(za=z_ref[0], zb=z_ref[1], lane16=lane16, grp16=grp16, odd=(grp16 & 1) == 1, hi=grp16 >= 2, tri=tri,
                    mbot=mbot, mtop=~mbot,
                    row8=lax.broadcasted_iota(jnp.int32, (8, 128), 0),
                    zero16=jnp.zeros((16, 128), u32))

    def qk(Q, g, C):
        lane16 = C["lane16"]
        lg = (80 * g + 80) % 128
        bias = jnp.where(lane16 == lg, jnp.uint32(ONE2), jnp.uint32(0))
        ss = []
        for r in range(4):
            q0 = mo(Q * (TB // 2) + 16 * r, 16)
            ws = []
            for j in range(4):
                f0 = DH * (4 * g + j)
                t, lo = f0 // 128, f0 % 128
                qt = q_ref[t, pl.ds(q0, 16), :]
                if lo + DH <= 128:
                    w = jnp.where((lane16 >= lo) & (lane16 < lo + DH), qt, bias)
                else:
                    qt1 = q_ref[t + 1, pl.ds(q0, 16), :]
                    w = jnp.where(lane16 >= lo, qt, jnp.where(lane16 < lo + DH - 128, qt1, bias))
                ws.append(w)
            wq = _b(_cat([ws[(gm - r) % 4] for gm in range(4)]))
            s = lax.dot_general(_b(km_ref[g, pl.ds(q0, 144), :]), wq, NTDIMS,
                                preferred_element_type=f32)
            mrg = jnp.where(C["tri"], s[256:288], s[0:32])
            mid = s[32:256]
            sbs[g % 2][r + C['za'], 0:224, :] = mid
            sbs[g % 2][r + C['za'], 224:256, :] = mrg
            ss.append(jnp.maximum(jnp.max(mid, axis=0, keepdims=True),
                                  jnp.max(mrg, axis=0, keepdims=True)))
        return ss

    def softmax(g, ms, C):
        zero16 = C["zero16"]
        sb, tb = sbs[g % 2], tbs[g % 2]

        def chunk(r, k):
            p = jnp.exp2(sb[r + C['zb'], 32 * k:32 * k + 32, :] - ms[r])
            return _cat([_pack2(p[0:8], p[8:16]), _pack2(p[16:24], p[24:32])])
        pw = [None] * 4
        for c in range(12):
            X = [None] * 4
            for r in range(4):
                k = c - r
                if k == 0:
                    pw[r] = chunk(r, 7)
                    X[r] = pw[r] & C["mtop"]
                elif k == 8:
                    X[r] = pw[r] & C["mbot"]
                elif 0 < k < 8:
                    X[r] = chunk(r, k - 1)
            nz = [r for r in range(4) if X[r] is not None]
            if len(nz) == 1:
                r = nz[0]
                T = [jnp.where(C["grp16"] == (j + r) % 4, X[r], zero16) for j in range(4)]
            else:
                def sel(mask, a, b):
                    if a is None and b is None:
                        return None
                    return jnp.where(mask, zero16 if a is None else a, zero16 if b is None else b)
                U = [sel(C["odd"], X[(p + 1) % 4], X[p]) for p in range(4)]
                Tp = [sel(C["hi"], U[(p + 2) % 4], U[p]) for p in range(4)]
                T = [zero16 if Tp[(-j) % 4] is None else Tp[(-j) % 4] for j in range(4)]
            for j in range(4):
                tb[j + C['za'], 16 * c:16 * c + 16, :] = T[j]

    def pv(Q, g, T, C):
        for j in range(4):
            h = 4 * g + j
            off = (DH * h) % 16
            base = DH * h - off
            r1 = (off + DH) % 32
            acc = None
            for t in range(3):
                v = vt_ref[Q + t, base // 2:base // 2 + 16, :]
                halves = [v[0:8], v[8:16]]
                hsel = (r1 // 2) // 8
                halves[hsel] = jnp.where(C["row8"] == (r1 // 2) % 8, jnp.uint32(ONE2), halves[hsel])
                vw = _b(_cat(halves))
                tt = _b(tbs[g % 2][j + C['zb'], 64 * t:64 * t + 64, :])
                d = jnp.dot(vw, tt, preferred_element_type=f32)
                acc = d if acc is None else acc + d
            linv = 1.0 / acc[r1:r1 + 1, :]
            lo8 = (off // 8) * 8
            o = acc[lo8:lo8 + 24, :] * linv
            if j:
                o = pltpu.roll(o, 128 - 32 * j, 1)
            ot_ref[DH * h:DH * h + DH, :] = o[off - lo8:off - lo8 + DH, :]

    def block(Q, par, mode):
        C = attn_consts()
        bstate = {}

        def U_pb(Qn, pn, n):
            return lambda: pb_unit(Qn, pn, n)

        def U_b(po, n):
            def f():
                bstate[n] = out_b(po, n)
            return f

        def U_a(Qo, n):
            return lambda: out_a(Qo, n, bstate.pop(n))

        if mode == "first":
            pbs = [U_pb(Q, par, n) for n in range(15)] + [U_pb(Q + 1, 1 - par, n) for n in range(15)]
            slots = [pbs[0:1], pbs[1:5], pbs[5:8], pbs[8:11], pbs[11:15], pbs[15:18], pbs[18:21],
                     pbs[21:24], pbs[24:28], pbs[28:30]]
        else:
            halo_copy(par)
            oa_transpose()
            battn(par, False)
            o = []
            for n in range(NT):
                o += [U_b(1 - par, n), U_a(Q - 1, n)]
            if mode == "mid":
                pbs = [U_pb(Q + 1, 1 - par, n) for n in range(15)]
                slots = [pbs[0:1], pbs[1:4],
                         [o[0], pbs[4], o[1]], [o[2], pbs[5]], [o[3], pbs[6], pbs[7]], [o[4], pbs[8]],
                         [o[5], pbs[9], pbs[10]], [o[6], pbs[11]],
                         [o[7], pbs[12], pbs[13], o[8]], [o[9], pbs[14]]]
            else:
                slots = [[], o[0:2], o[2:3], o[3:4], o[4:5], o[5:6], o[6:7], o[7:8], o[8:10], []]

        def run(us):
            for u in us:
                u()

        run(slots[0])
        ss = qk(Q, 0, C)
        run(slots[1])
        for g in range(NG):
            T = softmax(g, ss, C)
            if g + 1 < NG:
                ss = qk(Q, g + 1, C)
            else:
                pass
            if g + 1 < NG:
                pv(Q, g, T, C)
                run(slots[2 + g])
            else:
                pv(Q, g, T, C)
                run(slots[2 + g])
            if mode == "first" and g == 3:
                battn(par, True)
        if mode == "last":
            cp_o((NB - 2) * TB, TB, NB // 2 - 1).start()
            bs = [out_b(par, n) for n in range(NT)]
            oa_transpose()
            for n in range(NT):
                out_a(Q, n, bs[n])

    block(0, 0, "first")

    def p2(i, carry):
        block(2 * i + 1, 1, "mid")
        block(2 * i + 2, 0, "mid")
        cp_o(mo(2 * TB * i, 2 * TB), 2 * TB, i).start()
        return carry

    lax.fori_loop(0, (NB - 2) // 2, p2, 0)
    block(NB - 1, 1, "last")
    cp_o((NB - 1) * TB, TB, NB // 2).start()
    for i in range(NB // 2 - 1):
        cp_o(2 * TB * i, 2 * TB, i).wait()
    cp_o((NB - 2) * TB, TB, NB // 2 - 1).wait()
    cp_o((NB - 1) * TB, TB, NB // 2).wait()


@jax.jit
def pallas_gated_mix__sliding_block__sliding_local_dilated__prompt_kernel(A_x, A_wqkv, A_wo, B_x, B_wqkv, B_wo, gate_w):
    x = A_x.reshape(S, D)
    gw = gate_w.reshape(1, D)
    bbuf = [pltpu.VMEM((NT, TB, 128), f32), pltpu.VMEM((NT, 2, HALO + TB // 2, 128), f32),
            pltpu.VMEM((NT, 2, HALO + TB // 2, 128), f32)]
    out = pl.pallas_call(
        kernel,
        out_shape=jax.ShapeDtypeStruct((S, D), bf16),
        in_specs=[pl.BlockSpec(memory_space=pl.ANY)] * 6,
        out_specs=pl.BlockSpec(memory_space=pl.ANY),
        scratch_shapes=[
            pltpu.VMEM((S, D), bf16),
            pltpu.VMEM((3, D, D), bf16),
            pltpu.VMEM((D, D), bf16),
            pltpu.VMEM((3, D, D), bf16),
            pltpu.VMEM((D, D), bf16),
            pltpu.VMEM((1, D), bf16),
            pltpu.VMEM((S, D), bf16),
            pltpu.SemaphoreType.DMA((8,)),
            pltpu.SemaphoreType.DMA((3,)),
            pltpu.SemaphoreType.DMA((3,)),
            pltpu.SemaphoreType.DMA((NB // 2 + 1,)),
            pltpu.VMEM((S // 2, D), u32),
            pltpu.VMEM((S, 128), f32),
            pltpu.VMEM((NT, S // 2, 128), u32),
            pltpu.VMEM((NG, (WIN + S) // 2, 128), u32),
            pltpu.VMEM((NB + 2, D // 2, 128), u32),
            pltpu.VMEM((D // 2, D), u32),
            pltpu.VMEM((3 * D // 2, D), u32),
            pltpu.VMEM((D // 2, D), u32),
            pltpu.VMEM((D // 2, D), u32),
            pltpu.VMEM((NT, D // 2, 128), u32),
        ] + bbuf + bbuf + [
            pltpu.VMEM((D, 128), f32),
            pltpu.VMEM((TB // 2, D), u32),
            pltpu.VMEM((TB // 2, D), u32),
            pltpu.VMEM((TB // 2, D), u32),
            pltpu.VMEM((4, 256, 128), f32),
            pltpu.VMEM((4, 256, 128), f32),
            pltpu.VMEM((4, 192, 128), u32),
            pltpu.VMEM((4, 192, 128), u32),
            pltpu.SMEM((2,), jnp.int32),
        ],
        compiler_params=pltpu.CompilerParams(vmem_limit_bytes=100 * 1024 * 1024),
    )(x, A_wqkv, A_wo, B_wqkv, B_wo, gw)
    return out.reshape(1, S, D)
```

```python
import functools
import math

import jax
import jax.numpy as jnp
from jax import lax
from jax.experimental import pallas as pl
from jax.experimental.pallas import tpu as pltpu

S, D, H, DH = 2048, 640, 32, 20
WIN = 256
TB = 128
NB = S // TB
NT = D // 128
NG = 8
QSCALE = DH ** -0.5 * math.log2(math.e)
ONE2 = 0x3F803F80
NEG2 = 0xF149F149
HI = 0xFFFF0000
R1 = 256
R2 = 512
TIE_OFF = 16
REL_BACK = 1
BPOS = [4, 5, 6, 8]
BPOS2 = [2, 3, 4, 5, 5, 6, 7, 8]
POP_LAT = 130
SMT = 4
SM_GROUPS = []
_acc, _cur = 0, []
for _c in range(12):
    for _hf in range(2):
        _cur.append((_c, _hf))
        _acc += sum(1 for _r in range(4) if 0 <= _c - _r < 8)
        if _acc >= SMT:
            SM_GROUPS.append(_cur)
            _acc, _cur = 0, []
SM_GROUPS[-1] = SM_GROUPS[-1] + _cur
BF = [0.5, 0.6, 0.72, 0.99]
BF2 = [0.25, 0.35, 0.5, 0.6, 0.6, 0.7, 0.85, 0.99]
BPOS = [int(f * len(SM_GROUPS)) for f in BF]
BPOS2 = [int(f * len(SM_GROUPS)) for f in BF2]
WS = 350
WE = 100000
WV = 200
WP = 100000
HALO = 8
NTDIMS = (((1,), (1,)), ((), ()))

f32 = jnp.float32
bf16 = jnp.bfloat16
u32 = jnp.uint32


def _u(x):
    return pltpu.bitcast(x, u32)


def _b(x):
    return pltpu.bitcast(x, bf16)


def _f(x):
    return pltpu.bitcast(x, f32)


def _pack2(a, b):
    return (_u(a) >> 16) | (_u(b) & jnp.uint32(HI))


def _pack2r(a, b):
    h = jnp.uint32(0x8000)
    return ((_u(a) + h) >> 16) | ((_u(b) + h) & jnp.uint32(HI))


def _cat(xs):
    return jnp.concatenate(xs, axis=0)


def kernel(x_hbm, wa_hbm, woa_hbm, wb_hbm, wob_hbm, gw_hbm, o_hbm,
           x_ref, wa_ref, woa_ref, wb_ref, wob_ref, gw_ref, o_ref, sem_in, sem_x, sem_wb, sem_o,
           xm_ref, g_ref, q_ref, km_ref, vt_ref, wvt_ref, wbpt_ref, woau_ref, wobp_ref, tmp_ref,
           qb0, kb0, vb0, qb1, kb1, vb1, ot_ref, oa_ref, ob0, ob1, s0, s1, t0_, t1_, m_ref, z_ref):
    sbs, tbs = (s0, s1), (t0_, t1_)
    qbs, kbs, vbs, obs = (qb0, qb1), (kb0, kb1), (vb0, vb1), (ob0, ob1)

    def mo(v, m):
        return v if isinstance(v, int) else pl.multiple_of(v, m)

    def cp_x(r0, n, sem):
        return pltpu.make_async_copy(x_hbm.at[pl.ds(r0, n), :], x_ref.at[pl.ds(r0, n), :], sem)

    def cp_xl(p):
        return cp_x(mo(R2 * (p + 1), R2), R2, sem_x.at[p])

    def cp_wa(p):
        return pltpu.make_async_copy(wa_hbm.at[:, pl.ds(D * p, D)], wa_ref.at[p], sem_in.at[p])

    def cp_wb(p):
        return pltpu.make_async_copy(wb_hbm.at[:, pl.ds(mo(D * p, 128), D)], wb_ref.at[p], sem_wb.at[p])

    def cp_o(r0, n, k):
        return pltpu.make_async_copy(o_ref.at[pl.ds(r0, n), :], o_hbm.at[pl.ds(r0, n), :], sem_o.at[k])

    c_x0, c_x1 = cp_x(0, R1, sem_in.at[3]), cp_x(R1, R1, sem_in.at[4])
    c_gw = pltpu.make_async_copy(gw_hbm, gw_ref, sem_in.at[5])
    c_woa = pltpu.make_async_copy(woa_hbm, woa_ref, sem_in.at[6])
    c_wob = pltpu.make_async_copy(wob_hbm, wob_ref, sem_in.at[7])
    for c in (c_x0, cp_wa(0), c_gw, c_x1, cp_wa(2), cp_wa(1), cp_xl(0), cp_wb(0), cp_xl(1), cp_wb(1), cp_xl(2),
              cp_wb(2), c_woa, c_wob):
        c.start()

    z_ref[0] = 0
    z_ref[1] = 0
    z_ref[2] = 0

    def deint(src, dst, doff, cs):
        for e in range(DH // 2):
            rows = src[pl.ds(e, H, stride=DH // 2), :]
            a = _cat([rows[0:8], rows[16:24]])
            b = _cat([rows[8:16], rows[24:32]])
            lo = (a & jnp.uint32(0xFFFF)) | (b << 16)
            hi = (a >> 16) | (b & jnp.uint32(HI))
            dst[pl.ds(mo(doff + 32 * e, 16), 16), cs] = lo
            dst[pl.ds(mo(doff + 32 * e + 16, 16), 16), cs] = hi

    lane_p = lax.broadcasted_iota(jnp.int32, (WIN // 2, 128), 1)
    for g in range(NG):
        lg = (80 * g + 80) % 128
        km_ref[g, 0:WIN // 2, :] = jnp.where(lane_p == lg, jnp.uint32(NEG2), jnp.uint32(0))
    vt_ref[0:2] = jnp.zeros((2, D // 2, 128), u32)
    kb0[0:NT, :, 0:HALO, :] = jnp.zeros((NT, 2, HALO, 128), f32)
    vb0[0:NT, :, 0:HALO, :] = jnp.zeros((NT, 2, HALO, 128), f32)

    def p1_q(i):
        r0, h0 = mo(i * R1, R1), mo(i * (R1 // 2), R1 // 2)
        xb = x_ref[pl.ds(r0, R1), :]
        q = jnp.dot(xb, wa_ref[0], preferred_element_type=f32)
        for t in range(NT):
            q_ref[t, pl.ds(h0, R1 // 2), :] = _u((q[:, 128 * t:128 * t + 128] * QSCALE).astype(bf16))
        xw = _u(xb)
        ev = _f(xw << 16)
        od = _f(xw & jnp.uint32(HI))
        xm = _cat([z[8 * k:8 * k + 8] for k in range(R1 // 16) for z in (ev, od)])
        xm_ref[pl.ds(h0, R1 // 2), :] = _u(xm.astype(bf16))
        z = jnp.sum(xb.astype(f32) * gw_ref[...].astype(f32).reshape(1, D), axis=-1, keepdims=True)
        g_ref[pl.ds(r0, R1), :] = jnp.broadcast_to(jax.nn.sigmoid(z), (R1, 128))

    def p1_k(i):
        r0, h0 = mo(i * R1, R1), mo(i * (R1 // 2), R1 // 2)
        xb = x_ref[pl.ds(r0, R1), :]
        k = jnp.dot(xb, wa_ref[1], preferred_element_type=f32)
        kt = [_u(k[:, 128 * t:128 * t + 128].astype(bf16)) for t in range(NT)]
        lane = lax.broadcasted_iota(jnp.int32, (R1 // 2, 128), 1)
        for g in range(NG):
            t0 = (80 * g) // 128
            t1 = (80 * g + 79) // 128
            lg = (80 * g + 80) % 128
            v = jnp.where(lane == lg, jnp.uint32(0), kt[t0])
            if t1 != t0:
                v = jnp.where(lane < lg, kt[t1], v)
            km_ref[g, pl.ds(WIN // 2 + h0, R1 // 2), :] = v

    def p1_v(i):
        r0 = mo(i * R1, R1)
        xf = x_ref[pl.ds(r0, R1), :].astype(f32)
        xp = _cat([_pack2(xf[16 * k:16 * k + 8], xf[16 * k + 8:16 * k + 16]) for k in range(R1 // 16)])
        vt = lax.dot_general(_b(wvt_ref[...]), _b(xp), NTDIMS, preferred_element_type=f32)
        for c in range(R1 // 128):
            vt_ref[2 + i * (R1 // 128) + c] = _u(vt[:, 128 * c:128 * c + 128].astype(bf16))

    c_x0.wait()
    cp_wa(0).wait()
    c_gw.wait()
    p1_q(0)
    c_x1.wait()
    p1_q(1)
    cp_wa(2).wait()
    cp_wa(1).wait()
    for c in range(NT):
        cs = slice(128 * c, 128 * c + 128)
        wvt_ref[:, cs] = _u(wa_ref[2, cs, :].T)
    p1_k(0)
    p1_k(1)
    p1_v(0)
    p1_v(1)

    def p1(p, carry):
        cp_xl(p).wait()
        cp_wb(p).wait()
        for c in range(NT):
            cs = slice(128 * c, 128 * c + 128)
            tmp_ref[c] = _u(wb_ref[p, cs, :].T)
            deint(tmp_ref.at[c], wbpt_ref, 320 * p, cs)
        for i in (2 * p + 2, 2 * p + 3):
            p1_q(i)
            p1_k(i)
            p1_v(i)
        return carry

    lax.fori_loop(0, 3, p1, 0)

    c_woa.wait()
    c_wob.wait()
    for c in range(NT):
        cs = slice(128 * c, 128 * c + 128)
        tmp_ref[c] = _u(wob_ref[:, cs])
        deint(tmp_ref.at[c], wobp_ref, 0, cs)
        woau_ref[:, cs] = _u(woa_ref[:, cs])

    def tied(x, ties, C):
        for r8, kt, tok in ties:
            rs = slice(8 * r8, 8 * r8 + 8)
            parts = []
            if kt > 0:
                parts.append(x[rs, :128 * kt])
            parts.append(jnp.where(C["never"], tok, x[rs, 128 * kt:128 * kt + 128]))
            if 128 * kt + 128 < x.shape[1]:
                parts.append(x[rs, 128 * kt + 128:])
            rows = []
            if r8 > 0:
                rows.append(x[:8 * r8])
            rows.append(jnp.concatenate(parts, axis=1) if len(parts) > 1 else parts[0])
            if 8 * r8 + 8 < x.shape[0]:
                rows.append(x[8 * r8 + 8:])
            x = _cat(rows)
        return _b(x)

    def pb_pass(Qn, pn, n, k, st, ties, C):
        h0 = mo(Qn * (TB // 2), TB // 2)
        ks = slice(128 * k, 128 * k + 128)
        xb = tied(xm_ref[pl.ds(h0, TB // 2), ks], ties, C)
        w = _b(wbpt_ref[64 * n:64 * n + 64, ks])
        d = lax.dot_general(xb, w, NTDIMS, preferred_element_type=f32)
        res = st["acc"] = d if k == 0 else st["acc"] + d
        if k == NT - 1:
            p, t = n // NT, n % NT
            if p == 0:
                qbs[pn][t] = res * QSCALE
            else:
                dst = (kbs if p == 1 else vbs)[pn]
                for i in range(TB // 16):
                    for e in range(2):
                        dst[t, e, HALO + 8 * i:HALO + 8 * i + 8, :] = res[16 * i + 8 * e:16 * i + 8 * e + 8]
        return d

    def halo_copy(par):
        for bufs in (kbs, vbs):
            bufs[par][0:NT, :, 0:HALO, :] = bufs[1 - par][0:NT, :, TB // 2:TB // 2 + HALO, :]

    def oa_transpose():
        for t in range(NT):
            oa_ref[:, 128 * t:128 * t + 128] = _u(ot_ref[128 * t:128 * t + 128, :].astype(bf16).T)

    def ob_pass(po, n, k, st, ties, C):
        d = jnp.dot(tied(obs[po][0, :, 128 * k:128 * k + 128], ties, C),
                    _b(wobp_ref[64 * k:64 * k + 64, 128 * n:128 * n + 128]), preferred_element_type=f32)
        st["b"] = d if k == 0 else st["b"] + d
        return d

    def oa_pass(Qo, n, k, st, ties, C):
        d = jnp.dot(tied(oa_ref[:, 128 * k:128 * k + 128], ties, C),
                    _b(woau_ref[64 * k:64 * k + 64, 128 * n:128 * n + 128]), preferred_element_type=f32)
        a = st["a"] = d if k == 0 else st["a"] + d
        if k == NT - 1:
            r0 = mo(Qo * TB, TB)
            gate = g_ref[pl.ds(r0, TB), :]
            b = st["b"]
            o_ref[pl.ds(r0, TB), 128 * n:128 * n + 128] = (b + gate * (a - b)).astype(bf16)
        return d

    def battn_pieces(par, first, i, C):
        qb, kb, vb, ob = qbs[par], kbs[par], vbs[par], obs[par]
        st = {"ls": []}

        def win(buf, t, w):
            o = HALO + 8 * i - w
            return _cat([buf[t, 0, o:o + 8, :], buf[t, 1, o:o + 8, :]])

        def scores(ws):
            def f(rel):
                q = [qb[t, 16 * i:16 * i + 16, :] for t in range(NT)]
                if rel is not None:
                    q = [_cat([jnp.where(C["never"], rel, v[0:8]), jnp.where(C["never"], rel, v[8:16])]) for v in q]
                for w in ws:
                    acc = None
                    for t in range(NT):
                        pr = q[t] * win(kb, t, w)
                        acc = pr if acc is None else acc + pr
                    acc = acc + pltpu.roll(acc, 64, 1)
                    acc = acc + pltpu.roll(acc, 32, 1)
                    if first and i == 0 and w > 0:
                        pos = lax.broadcasted_iota(jnp.int32, (16, 128), 0) & 7
                        acc = jnp.where(pos >= w, acc, -1e30)
                    st["ls"].append(acc)
                    st["m"] = acc if w == 0 else jnp.maximum(st["m"], acc)
                return _u(st["m"][0:8])
            return f

        def exps(rel):
            m = st["m"]
            if rel is not None:
                m = _cat([jnp.where(C["never"], rel, m[0:8]), jnp.where(C["never"], rel, m[8:16])])
            st["ps"] = [jnp.exp2(l - m) for l in st["ls"]]
            st["linv"] = 1.0 / functools.reduce(lambda a, b: a + b, st["ps"])
            return _u(st["linv"][0:8])

        def pvs(ts):
            def f(rel):
                if rel is not None:
                    vb[NT + C["za"], 0, 0:8, :] = rel
                tok = None
                for t in ts:
                    acc = None
                    for w in range(8):
                        pr = st["ps"][w] * win(vb, t, w)
                        acc = pr if acc is None else acc + pr
                    acc = acc * st["linv"]
                    o = _pack2r(acc[0:8], acc[8:16])
                    ob[0, 8 * i:8 * i + 8, 128 * t:128 * t + 128] = o
                    tok = o if tok is None else tok | o
                return tok
            return f
        return [(scores(list(range(8))), WS), (exps, WE), (pvs([0, 1, 2]), WV), (pvs([3, 4]), WV)]

    def attn_consts():
        lane16 = lax.broadcasted_iota(jnp.int32, (16, 128), 1)
        grp8 = lax.broadcasted_iota(jnp.int32, (8, 128), 1) // 32
        row32 = lax.broadcasted_iota(jnp.int32, (32, 128), 0)
        lane32 = lax.broadcasted_iota(jnp.int32, (32, 128), 1)
        tri = row32 <= (lane32 & 31)
        ones = jnp.full((32, 128), -1, jnp.int32)
        tb = _f(jnp.where(tri, ones, 0))
        mbot = _cat([_pack2(tb[0:8], tb[8:16]), _pack2(tb[16:24], tb[24:32])])
        return dict(za=z_ref[0], zb=z_ref[1], lane16=lane16, grp8=grp8, odd=(grp8 & 1) == 1, hi=grp8 >= 2,
                    tri=tri, mbot=mbot, mtop=~mbot,
                    never=lax.broadcasted_iota(jnp.int32, (8, 128), 1) < z_ref[2],
                    row8=lax.broadcasted_iota(jnp.int32, (8, 128), 0),
                    zero16=jnp.zeros((16, 128), u32))

    def qk_r(Q, g, r, ties, C):
        lane16 = C["lane16"]
        lg = (80 * g + 80) % 128
        bias = jnp.where(lane16 == lg, jnp.uint32(ONE2), jnp.uint32(0))
        q0 = mo(Q * (TB // 2) + 16 * r, 16)
        ws = []
        for j in range(4):
            f0 = DH * (4 * g + j)
            t, lo = f0 // 128, f0 % 128
            qt = q_ref[t, pl.ds(q0, 16), :]
            if lo + DH <= 128:
                w = jnp.where((lane16 >= lo) & (lane16 < lo + DH), qt, bias)
            else:
                qt1 = q_ref[t + 1, pl.ds(q0, 16), :]
                w = jnp.where(lane16 >= lo, qt, jnp.where(lane16 < lo + DH - 128, qt1, bias))
            ws.append(w)
        wq = _b(_cat([ws[(gm - r) % 4] for gm in range(4)]))
        s = lax.dot_general(tied(km_ref[g, pl.ds(q0, 144), :], ties, C), wq, NTDIMS,
                            preferred_element_type=f32)
        mrg = jnp.where(C["tri"], s[256:288], s[0:32])
        mid = s[32:256]
        sbs[g % 2][r + C['za'], 0:224, :] = mid
        sbs[g % 2][r + C['za'], 224:256, :] = mrg
        return s, jnp.maximum(jnp.max(mid, axis=0, keepdims=True), jnp.max(mrg, axis=0, keepdims=True))

    def softmax_pieces(g, ms, C):
        zero8 = C["zero16"][0:8]
        sb, tb = sbs[g % 2], tbs[g % 2]
        pw = {}

        def chunk(r, k, hf):
            o = 32 * k + 16 * hf
            p = jnp.exp2(sb[r + C['zb'], o:o + 16, :] - ms[r])
            return _pack2(p[0:8], p[8:16])

        def col(c, hf):
            hs = slice(8 * hf, 8 * hf + 8)
            X = [None] * 4
            for r in range(4):
                k = c - r
                if k == 0:
                    pw[r, hf] = chunk(r, 7, hf)
                    X[r] = pw[r, hf] & C["mtop"][hs]
                elif k == 8:
                    X[r] = pw[r, hf] & C["mbot"][hs]
                elif 0 < k < 8:
                    X[r] = chunk(r, k - 1, hf)
            nz = [r for r in range(4) if X[r] is not None]
            if len(nz) == 1:
                r = nz[0]
                T = [jnp.where(C["grp8"] == (j + r) % 4, X[r], zero8) for j in range(4)]
            else:
                def sel(mask, a, b):
                    if a is None and b is None:
                        return None
                    return jnp.where(mask, zero8 if a is None else a, zero8 if b is None else b)
                U = [sel(C["odd"], X[(p + 1) % 4], X[p]) for p in range(4)]
                Tp = [sel(C["hi"], U[(p + 2) % 4], U[p]) for p in range(4)]
                T = [zero8 if Tp[(-j) % 4] is None else Tp[(-j) % 4] for j in range(4)]
            for j in range(4):
                tb[j + C['za'], 16 * c + 8 * hf:16 * c + 8 * hf + 8, :] = T[j]
            return T[0]

        def piece(cs):
            def f(rel):
                if rel is not None:
                    sb[4 + C['za'], 0:8, :] = rel
                return functools.reduce(lambda a, b: a | b, [col(c, hf) for c, hf in cs])
            return f
        return [(piece(cs), WP) for cs in SM_GROUPS]

    def pv_j(Q, g, j, C):
        h = 4 * g + j
        off = (DH * h) % 16
        base = DH * h - off
        r1 = (off + DH) % 32
        acc = None
        for t in range(3):
            v = vt_ref[Q + t, base // 2:base // 2 + 16, :]
            halves = [v[0:8], v[8:16]]
            hsel = (r1 // 2) // 8
            halves[hsel] = jnp.where(C["row8"] == (r1 // 2) % 8, jnp.uint32(ONE2), halves[hsel])
            vw = _b(_cat(halves))
            tt = _b(tbs[g % 2][j + C['zb'], 64 * t:64 * t + 64, :])
            d = jnp.dot(vw, tt, preferred_element_type=f32)
            acc = d if acc is None else acc + d
        linv = 1.0 / acc[r1:r1 + 1, :]
        lo8 = (off // 8) * 8
        o = acc[lo8:lo8 + 24, :] * linv
        if j:
            o = pltpu.roll(o, 128 - 32 * j, 1)
        ot_ref[DH * h:DH * h + DH, :] = o[off - lo8:off - lo8 + DH, :]

    def section(specs):
        C = attn_consts()
        clock = [0, 0, 0, 0]
        reg = []

        def place(rows):
            m = clock.index(min(clock))
            s = clock[m]
            clock[m] += rows
            return s

        def U_pb(Qn, pn, n):
            st = {}
            return [functools.partial(pb_pass, Qn, pn, n, k, st) for k in range(NT)]

        def U_o(po, Qo, n):
            st = {}
            return ([functools.partial(ob_pass, po, n, k, st) for k in range(NT)],
                    [functools.partial(oa_pass, Qo, n, k, st) for k in range(NT)])

        def token(tm):
            best = None
            for lo, rows, res in reg:
                if lo <= tm:
                    r = min((tm - lo) // 8, rows // 8 - 1)
                    if best is None or lo + 8 * r >= best[0]:
                        best = (lo + 8 * r, res, r)
            return None if best is None else best[1][8 * best[2]:8 * best[2] + 8]

        def plain(units):
            for u in units:
                for f in u:
                    t0 = place(128)
                    reg.append((t0 + POP_LAT, 128, f([], C)))

        ms = None
        for bi, (Q, par, mode) in enumerate(specs):
            tail = bi == len(specs) - 1
            if mode == "first":
                F = [U_pb(Q, par, n) for n in range(15)] + [U_pb(Q + 1, 1 - par, n) for n in range(15)]
                plain(F[0:1])
                ms = []
                for r in range(4):
                    place(288)
                    ms.append(qk_r(Q, 0, r, [], C)[1])
                plain(F[1:3])
                F = F[3:]
                cnt = [4, 4, 4, 3, 3, 3, 3, 3]
            else:
                o = []
                for n in range(NT):
                    o += list(U_o(1 - par, Q - 1, n))
                if mode == "mid":
                    p = [U_pb(Q + 1, 1 - par, n) for n in range(15)]
                    F = [p[0], p[1], p[2], p[3], p[4], p[5], o[0], o[1], p[6], o[2], o[3], p[7], o[4], o[5], p[8],
                         o[6], o[7], p[9], o[8], o[9], p[10], p[11], p[12], p[13], p[14]]
                    cnt = [3, 3, 3, 3, 3, 3, 3, 4]
                else:
                    F = o
                    cnt = [1, 1, 1, 1, 1, 1, 2, 2]
                halo_copy(par)
                if bi == 0:
                    ms = [m_ref[r, 0:1, :] for r in range(4)]
            assert sum(cnt) == len(F)
            k = 0
            for g in range(NG):
                fl = [f for u in F[k:k + cnt[g]] for f in u]
                k += cnt[g]
                P = softmax_pieces(g, ms, C)
                if mode != "first":
                    B = battn_pieces(par, False, g, C)
                elif g >= 4:
                    B = battn_pieces(par, True, 2 * g - 8, C) + battn_pieces(par, True, 2 * g - 7, C)
                else:
                    B = []
                seq = []
                bpos = BPOS if len(B) == 4 else BPOS2
                for ip, pc in enumerate(P):
                    seq.append(pc)
                    for ib, bc in enumerate(B):
                        if bpos[ib] == ip:
                            seq.append(bc)
                has_qk = not (mode == "last" and g == NG - 1)
                has_pv = not (mode == "first" and g == 0)
                Qn, gn = (Q, g + 1) if g + 1 < NG else (Q + 1, 0)
                Qp, gp = (Q, g - 1) if g > 0 else (Q - 1, NG - 1)
                tbeg = min(clock)
                passes = []
                if has_qk:
                    passes += [("q", r, place(288), 288) for r in range(4)]
                if has_pv:
                    passes += [("p", j, [place(32) for _ in range(3)][0], 0) for j in range(4)]
                passes += [("f", u, place(128), 128) for u in range(len(fl))]
                tend = min(clock)
                slots = {}
                lastp = 0
                dl = []
                for s, pc in enumerate(seq):
                    tm = tbeg + (s + 1) * (tend - tbeg) // len(seq) - TIE_OFF
                    cand = [ip for ip, (kd, _, t0, rows) in enumerate(passes)
                            if ip >= lastp and rows and t0 <= tm < t0 + rows]
                    if not cand:
                        cand = [ip for ip, (kd, _, t0, rows) in enumerate(passes)
                                if ip >= lastp and rows and t0 > tm][:1]
                    if not cand:
                        cand = [len(passes) - 1]
                    ip = cand[0]
                    lastp = ip
                    t0, rows = passes[ip][2], passes[ip][3]
                    r8 = min(max(tm - t0, 0) // 16, rows // 16 - 1)
                    while any(x[1] == r8 for x in slots.get(ip, [])) and r8 < rows // 16 - 1:
                        r8 += 1
                    slots.setdefault(ip, []).append((s, r8))
                    dl.append(t0 + 16 * r8)
                ms_n = []
                for ip, (kd, idx, t0, rows) in enumerate(passes):
                    ties = []
                    for s, r8 in slots.get(ip, []):
                        ties.append((r8, 0, seq[s][0](token(dl[s] - seq[s][1]))))
                    if kd == "q":
                        sres, m = qk_r(Qn, gn, idx, ties, C)
                        ms_n.append(m)
                        reg.append((t0 + POP_LAT, rows, sres))
                        if g + 1 == NG and tail:
                            m_ref[idx] = jnp.broadcast_to(m, (8, 128))
                    elif kd == "p":
                        pv_j(Qp, gp, idx, C)
                        if g == 0 and idx == 3:
                            oa_transpose()
                    else:
                        reg.append((t0 + POP_LAT, rows, fl[idx](ties, C)))
                ms = ms_n
            if mode == "last":
                cp_o((NB - 2) * TB, TB, NB // 2 - 1).start()
                o = [U_o(par, Q, n) for n in range(NT)]
                plain([u[0] for u in o])
                for j in range(4):
                    pv_j(Q, NG - 1, j, C)
                oa_transpose()
                plain([u[1] for u in o])

    section([(0, 0, "first")])

    def p2(i, carry):
        section([(2 * i + 1, 1, "mid"), (2 * i + 2, 0, "mid")])
        cp_o(mo(2 * TB * i, 2 * TB), 2 * TB, i).start()
        return carry

    lax.fori_loop(0, (NB - 2) // 2, p2, 0)
    section([(NB - 1, 1, "last")])
    cp_o((NB - 1) * TB, TB, NB // 2).start()
    for i in range(NB // 2 - 1):
        cp_o(2 * TB * i, 2 * TB, i).wait()
    cp_o((NB - 2) * TB, TB, NB // 2 - 1).wait()
    cp_o((NB - 1) * TB, TB, NB // 2).wait()


@jax.jit
def pallas_gated_mix__sliding_block__sliding_local_dilated__prompt_kernel(A_x, A_wqkv, A_wo, B_x, B_wqkv, B_wo, gate_w):
    x = A_x.reshape(S, D)
    gw = gate_w
    bbuf = [pltpu.VMEM((NT, TB, 128), f32), pltpu.VMEM((NT + 1, 2, HALO + TB // 2, 128), f32),
            pltpu.VMEM((NT + 1, 2, HALO + TB // 2, 128), f32)]
    out = pl.pallas_call(
        kernel,
        out_shape=jax.ShapeDtypeStruct((S, D), bf16),
        in_specs=[pl.BlockSpec(memory_space=pl.ANY)] * 6,
        out_specs=pl.BlockSpec(memory_space=pl.ANY),
        scratch_shapes=[
            pltpu.VMEM((S, D), bf16),
            pltpu.VMEM((3, D, D), bf16),
            pltpu.VMEM((D, D), bf16),
            pltpu.VMEM((3, D, D), bf16),
            pltpu.VMEM((D, D), bf16),
            pltpu.VMEM((D,), bf16),
            pltpu.VMEM((S, D), bf16),
            pltpu.SemaphoreType.DMA((8,)),
            pltpu.SemaphoreType.DMA((3,)),
            pltpu.SemaphoreType.DMA((3,)),
            pltpu.SemaphoreType.DMA((NB // 2 + 1,)),
            pltpu.VMEM((S // 2, D), u32),
            pltpu.VMEM((S, 128), f32),
            pltpu.VMEM((NT, S // 2, 128), u32),
            pltpu.VMEM((NG, (WIN + S) // 2, 128), u32),
            pltpu.VMEM((NB + 2, D // 2, 128), u32),
            pltpu.VMEM((D // 2, D), u32),
            pltpu.VMEM((3 * D // 2, D), u32),
            pltpu.VMEM((D // 2, D), u32),
            pltpu.VMEM((D // 2, D), u32),
            pltpu.VMEM((NT, D // 2, 128), u32),
        ] + bbuf + bbuf + [
            pltpu.VMEM((D, 128), f32),
            pltpu.VMEM((TB // 2, D), u32),
            pltpu.VMEM((1, TB // 2, D), u32),
            pltpu.VMEM((1, TB // 2, D), u32),
            pltpu.VMEM((5, 256, 128), f32),
            pltpu.VMEM((5, 256, 128), f32),
            pltpu.VMEM((4, 192, 128), u32),
            pltpu.VMEM((4, 192, 128), u32),
            pltpu.VMEM((4, 8, 128), f32),
            pltpu.SMEM((3,), jnp.int32),
        ],
        compiler_params=pltpu.CompilerParams(vmem_limit_bytes=100 * 1024 * 1024),
    )(x, A_wqkv, A_wo, B_wqkv, B_wo, gw)
    return out.reshape(1, S, D)
```

```python
import functools
import math

import jax
import jax.numpy as jnp
from jax import lax
from jax.experimental import pallas as pl
from jax.experimental.pallas import tpu as pltpu

S, D, H, DH = 2048, 640, 32, 20
TB = 128
NB = S // TB
NT = D // 128
NG = 8
QSCALE = DH ** -0.5 * math.log2(math.e)
ONE2 = 0x3F803F80
HI = 0xFFFF0000
TIE_OFF = 16
POP_LAT = 130
SMT = 4
SM_GROUPS = []
_acc, _cur = 0, []
for _c in range(12):
    for _hf in range(2):
        _cur.append((_c, _hf))
        _acc += sum(1 for _r in range(4) if 0 <= _c - _r < 8)
        if _acc >= SMT:
            SM_GROUPS.append(_cur)
            _acc, _cur = 0, []
SM_GROUPS[-1] = SM_GROUPS[-1] + _cur
BF = [0.5, 0.6, 0.72, 0.99]
BF2 = [0.25, 0.35, 0.5, 0.6, 0.6, 0.7, 0.85, 0.99]
XF = 0.3
WS = 350
WE = 100000
WV = 200
WP = 100000
HOOK = 1
WAITS = {2: [2], 3: [3, 4], 5: [5, 6, 7], 8: [8, 9]}
B0CNT = [2, 2, 2, 2, 2, 3, 2, 3]
B1CNT = [3, 3, 3, 3, 3, 3, 2, 5]
CUCNT = [2, 2, 2, 2, 2, 2, 2, 2, 2, 2, 2, 2, 2, 2, 1, 1]
DCNT = [2, 3, 2, 3, 2, 3, 2, 3]
B01CNT = [3, 3, 3, 3, 3, 3, 2, 2, 2, 2, 2, 2, 2, 2, 2, 2]
B1POS = [0, 1, 2, 3, 4, 5, 6, 7, 8, 9, 10, 12, 13, 15]
P6 = 5
P7 = 2
PB1 = 3
PB2 = 2
XN = 3
WX = 350
PVD = 750
WM = 200
ORD = "bbbbb bbboo bboov kboov qkoov qkbvo qkbvo qkqbb"
HALO = 8
NTDIMS = (((1,), (1,)), ((), ()))

f32 = jnp.float32
bf16 = jnp.bfloat16
u32 = jnp.uint32


def _u(x):
    return pltpu.bitcast(x, u32)


def _b(x):
    return pltpu.bitcast(x, bf16)


def _f(x):
    return pltpu.bitcast(x, f32)


def _pack2(a, b):
    return (_u(a) >> 16) | (_u(b) & jnp.uint32(HI))


def _pack2r(a, b):
    h = jnp.uint32(0x8000)
    return ((_u(a) + h) >> 16) | ((_u(b) + h) & jnp.uint32(HI))


def _cat(xs):
    return jnp.concatenate(xs, axis=0)


class Blk:
    def __init__(self, i, off, cache=None):
        self.i, self.off, self.cache = i, off, ({} if cache is None else cache)

    def __add__(self, k):
        return Blk(self.i, self.off + k, self.cache)

    def at(self, per, extra=0):
        c = self.off * per + extra
        if self.i is None:
            return c
        if per not in self.cache:
            self.cache[per] = self.i * (2 * per)
        al = math.gcd(2 * per, c)
        v = self.cache[per] + c
        return pl.multiple_of(v, al) if al > 1 else v

    @property
    def cmin(self):
        return max(0, 8 - 4 * self.off) if self.i is None else 0


def kernel(x_hbm, wa_hbm, woa_hbm, wb_hbm, wob_hbm, gw_hbm, o_hbm,
           x_ref, wqk_ref, wv_ref, woa_ref, wb_ref, wob_ref, gw_ref, o_ref, sem,
           wu_ref, xu_ref, xm_ref, g_ref, q_ref, km_ref, vt_ref, wvt_ref, wbpt_ref, wobp_ref, tmp_ref,
           qb0, kb0, vb0, qb1, kb1, vb1, qb2, kb2, vb2, ot_ref, oa0, oa1, ob0, ob1, ob2, s0, s1, t0_, t1_, m_ref, z_ref):
    sbs, tbs = (s0, s1), (t0_, t1_)
    qbs, kbs, vbs, obs, oas = (qb0, qb1, qb2), (kb0, kb1, kb2), (vb0, vb1, vb2), (ob0, ob1, ob2), (oa0, oa1)

    def cp_x(r0, n, k):
        return pltpu.make_async_copy(x_hbm.at[pl.ds(r0, n), :], x_ref.at[pl.ds(r0, n), :], sem.at[k])

    def cp_w(n, k):
        return pltpu.make_async_copy(wa_hbm.at[:, pl.ds(128 * n, 128)], wqk_ref.at[n], sem.at[k])

    def cp_wb(p):
        return pltpu.make_async_copy(wb_hbm.at[:, pl.ds(D * p, D)], wb_ref.at[p], sem.at[(4, 0, 0)[p]])

    def cp_woa(n):
        return pltpu.make_async_copy(woa_hbm.at[:, pl.ds(128 * n, 128)], woa_ref.at[n], sem.at[2])

    def cp_o(r0, n, k):
        return pltpu.make_async_copy(o_ref.at[pl.ds(r0, n), :], o_hbm.at[pl.ds(r0, n), :], sem.at[4])

    c_x = cp_x(0, 4 * TB, 0)
    c_xl = cp_x(4 * TB, S - 4 * TB, 3)
    c_gw = pltpu.make_async_copy(gw_hbm, gw_ref, sem.at[2])
    c_wv = pltpu.make_async_copy(wa_hbm.at[:, pl.ds(2 * D, D)], wv_ref, sem.at[1])
    c_wob = pltpu.make_async_copy(wob_hbm, wob_ref, sem.at[2])
    WORD = [0, 5, 1, 6, 2, 7, 3, 8, 4, 9]
    cw = [cp_w(n, k) for n, k in zip(WORD, [1, 2, 2, 3, 3, 3, 3, 4, 4, 4])]
    for c in [c_x, cw[0], c_gw] + cw[1:7] + [cp_wb(0)] + cw[7:]:
        c.start()

    z_ref[0] = 0
    z_ref[1] = 0
    z_ref[2] = 0
    kb2[0:NT, :, 0:HALO, :] = jnp.zeros((NT, 2, HALO, 128), f32)
    vb2[0:NT, :, 0:HALO, :] = jnp.zeros((NT, 2, HALO, 128), f32)
    vt_ref[0, D // 2 - 48:D // 2, :] = jnp.zeros((48, 128), u32)
    t1_[:, 0:64, :] = jnp.zeros((4, 64, 128), u32)

    def deint(src, dst, doff, cs):
        tok = None
        for e in range(DH // 2):
            rows = src[pl.ds(e, H, stride=DH // 2), :]
            a = _cat([rows[0:8], rows[16:24]])
            b = _cat([rows[8:16], rows[24:32]])
            lo = (a & jnp.uint32(0xFFFF)) | (b << 16)
            hi = (a >> 16) | (b & jnp.uint32(HI))
            dst[doff + 32 * e:doff + 32 * e + 16, cs] = lo
            dst[doff + 32 * e + 16:doff + 32 * e + 32, cs] = hi
            tok = hi[8:16] if tok is None else tok | hi[8:16]
        return tok

    def gated(w, rel):
        if rel is None:
            return w
        never = lax.broadcasted_iota(jnp.int32, (8, 128), 1) < z_ref[2]
        z = jnp.where(never, _u(rel), jnp.uint32(0))
        return w | jnp.tile(z, (w.shape[0] // 8, w.shape[1] // 128))

    def prep_wb(p, c):
        def f(rel):
            cs = slice(128 * c, 128 * c + 128)
            tmp_ref[c] = _u(_b(gated(_u(wb_ref[p, cs, :]), rel)).T)
            return deint(tmp_ref.at[c], wbpt_ref, 320 * p, cs)
        return (f, WX)

    def prep_wob(c):
        def f(rel):
            cs = slice(128 * c, 128 * c + 128)
            tmp_ref[c] = gated(_u(wob_ref[:, cs]), rel)
            return deint(tmp_ref.at[c], wobp_ref, 0, cs)
        return (f, WX)

    def prep_wv(c):
        def f(rel):
            cs = slice(128 * c, 128 * c + 128)
            w = _u(_b(gated(_u(wv_ref[cs, :]), rel)).T)
            wvt_ref[:, cs] = w
            return functools.reduce(lambda a, b: a | b, [w[64 * i + 56:64 * i + 64] for i in range(NT)])
        return (f, WX)

    def xm_piece(Q, i):
        def f(rel):
            r0, h0 = Q.at(TB, 32 * i), Q.at(TB // 2, 16 * i)
            xw = _u(x_ref[pl.ds(r0, 32), :])
            tok = None
            for t in range(NT):
                xu_ref[t, pl.ds(h0, 16), :] = xw[:, 128 * t:128 * t + 128]
                src = xu_ref.at[t, pl.ds(h0, 16), :]
                a = src[pl.ds(0, 8, stride=2), :]
                b = src[pl.ds(1, 8, stride=2), :]
                lo = (a & jnp.uint32(0xFFFF)) | (b << 16)
                hi = (a >> 16) | (b & jnp.uint32(HI))
                xm_ref[t, pl.ds(h0, 16), :] = _cat([lo, hi])
                tok = (lo | hi) if tok is None else tok | lo | hi
            return tok
        return (f, WP)

    def g_piece(Q, i):
        def f(rel):
            r0, h0 = Q.at(TB, 32 * i), Q.at(TB // 2, 16 * i)
            gw = gw_ref[...].astype(f32).reshape(1, D)
            z = None
            for t in range(NT):
                xb = _b(xu_ref[t, pl.ds(h0, 16), :]).astype(f32) * gw[:, 128 * t:128 * t + 128]
                z = xb if z is None else z + xb
            z = jnp.sum(z, axis=-1, keepdims=True)
            g = jnp.broadcast_to(jax.nn.sigmoid(z), (32, 128))
            g_ref[pl.ds(r0, 32), :] = g
            return _u(g[0:8]) | _u(g[8:16]) | _u(g[16:24]) | _u(g[24:32])
        return (f, WP)

    def tied(x, ties, C):
        for r8, tok in ties:
            rows = []
            if r8 > 0:
                rows.append(x[:8 * r8])
            rows.append(jnp.where(C["never"], tok, x[8 * r8:8 * r8 + 8]))
            if 8 * r8 + 8 < x.shape[0]:
                rows.append(x[8 * r8 + 8:])
            x = _cat(rows)
        return _b(x)

    def nat(res):
        return _cat([_pack2r(res[32 * i:32 * i + 16], res[32 * i + 16:32 * i + 32]) for i in range(TB // 32)])

    def qk_pass(Q, n, k, st, ties, C):
        h0 = Q.at(TB // 2)
        xb = tied(xm_ref[k, pl.ds(h0, TB // 2), :], ties, C)
        w = wqk_ref[n, 128 * k:128 * k + 128, :] if Q.i is None else _b(wu_ref[n, 64 * k:64 * k + 64, :])
        if Q.i is None and Q.off == 3:
            wu_ref[n, 64 * k:64 * k + 64, :] = _u(w)
        d = jnp.dot(xb, w, preferred_element_type=f32)
        res = st["acc"] = d if k == 0 else st["acc"] + d
        if k == NT - 1:
            if n < NT:
                q_ref[n, pl.ds(h0, TB // 2), :] = nat(res * QSCALE)
            else:
                t = n - NT
                kt = nat(res)
                for g in range(NG):
                    t0, t1, lg = (80 * g) // 128, (80 * g + 79) // 128, (80 * g + 80) % 128
                    if t0 == t1 == t:
                        km_ref[g, pl.ds(h0, TB // 2), :] = kt
                    elif t0 == t:
                        km_ref[g, pl.ds(h0, TB // 2), lg:128] = kt[:, lg:128]
                    elif t1 == t:
                        km_ref[g, pl.ds(h0, TB // 2), 0:lg] = kt[:, 0:lg]
        return d

    def v_pass(Q, n, k, st, ties, C):
        lhs = tied(wvt_ref[64 * n:64 * n + 64, 128 * k:128 * k + 128], ties, C)
        w = _b(xu_ref[k, pl.ds(Q.at(TB // 2), TB // 2), :])
        d = lax.dot_general(lhs, w, NTDIMS, preferred_element_type=f32)
        res = st["acc"] = d if k == 0 else st["acc"] + d
        if k == NT - 1:
            vt_ref[Q.at(1, 1), 64 * n:64 * n + 64, :] = _u(res.astype(bf16))
        return d

    def pb_pass(Q, pn, n, k, st, ties, C):
        xb = tied(xm_ref[k, pl.ds(Q.at(TB // 2), TB // 2), :], ties, C)
        w = _b(wbpt_ref[64 * n:64 * n + 64, 128 * k:128 * k + 128])
        d = lax.dot_general(xb, w, NTDIMS, preferred_element_type=f32)
        res = st["acc"] = d if k == 0 else st["acc"] + d
        if k == NT - 1:
            p, t = n // NT, n % NT
            if p == 0:
                qbs[pn][t] = res * QSCALE
            else:
                dst = (kbs if p == 1 else vbs)[pn]
                for i in range(TB // 32):
                    for e in range(2):
                        dst[t, e, HALO + 16 * i:HALO + 16 * i + 16, :] = res[32 * i + 16 * e:32 * i + 16 * e + 16]
        return d

    def halo_copy(par, src=None):
        for bufs in (kbs, vbs):
            bufs[par][0:NT, :, 0:HALO, :] = bufs[1 - par if src is None else src][0:NT, :, TB // 2:TB // 2 + HALO, :]

    def oa_transpose(oa, ts=range(NT)):
        for t in ts:
            oa[:, 128 * t:128 * t + 128] = _u(ot_ref[128 * t:128 * t + 128, :].astype(bf16).T)

    def ob_pass(ob, n, k, st, ties, C):
        d = jnp.dot(tied(ob[C['zb'], :, 128 * k:128 * k + 128], ties, C),
                    _b(wobp_ref[64 * k:64 * k + 64, 128 * n:128 * n + 128]), preferred_element_type=f32)
        st["b"] = d if k == 0 else st["b"] + d
        return d

    def oa_pass(Qo, oa, n, k, st, ties, C):
        if Qo.i is None and Qo.off == 0:
            w = woa_ref[n, 128 * k:128 * k + 128, :]
            wu_ref[10 + n, 64 * k:64 * k + 64, :] = _u(w)
        else:
            w = _b(wu_ref[10 + n, 64 * k:64 * k + 64, :])
        d = jnp.dot(tied(oa[:, 128 * k:128 * k + 128], ties, C), w, preferred_element_type=f32)
        a = st["a"] = d if k == 0 else st["a"] + d
        if k == NT - 1:
            r0 = Qo.at(TB)
            gate = g_ref[pl.ds(r0, TB), :]
            b = st["b"]
            o_ref[pl.ds(r0, TB), 128 * n:128 * n + 128] = (b + gate * (a - b)).astype(bf16)
        return d

    def oa_early(Qo, oa, n, k, st, ties, C):
        d = jnp.dot(tied(oa[:, 128 * k:128 * k + 128], ties, C), _b(wu_ref[10 + n, 64 * k:64 * k + 64, :]),
                    preferred_element_type=f32)
        a = st["a"] = d if k == 0 else st["a"] + d
        if k == NT - 2:
            b = st["b"]
            qb0[n] = b + g_ref[pl.ds(Qo.at(TB), TB), :] * (a - b)
        return d

    def oa_late(Qo, oa, n, ties, C):
        k, r0 = NT - 1, Qo.at(TB)
        d = jnp.dot(tied(oa[:, 128 * k:128 * k + 128], ties, C), _b(wu_ref[10 + n, 64 * k:64 * k + 64, :]),
                    preferred_element_type=f32)
        o_ref[pl.ds(r0, TB), 128 * n:128 * n + 128] = (qb0[n] + g_ref[pl.ds(r0, TB), :] * d).astype(bf16)
        return d

    def unit(fn, *args):
        st = {}
        return [functools.partial(fn, *args, k, st) for k in range(NT)]

    def U_o(Qo, oa, ob):
        us = []
        for n in range(NT):
            st = {}
            us.append([functools.partial(ob_pass, ob, n, k, st) for k in range(NT)])
            us.append([functools.partial(oa_pass, Qo, oa, n, k, st) for k in range(NT)])
        return us

    def battn_pieces(par, ob, first, i, C):
        qb, kb, vb = qbs[par], kbs[par], vbs[par]
        st = {"ls": []}
        q0 = 32 * (i // 2) + 8 * (i % 2)

        def win(buf, t, w):
            o = HALO + 8 * i - w
            return _cat([buf[t, 0, o:o + 8, :], buf[t, 1, o:o + 8, :]])

        def scores(rel):
            q = [[qb[t, q0:q0 + 8, :], qb[t, q0 + 16:q0 + 24, :]] for t in range(NT)]
            if rel is not None:
                q = [[jnp.where(C["never"], rel, v) for v in vv] for vv in q]
            q = [_cat(vv) for vv in q]
            for w in range(8):
                acc = None
                for t in range(NT):
                    pr = q[t] * win(kb, t, w)
                    acc = pr if acc is None else acc + pr
                acc = acc + pltpu.roll(acc, 64, 1)
                acc = acc + pltpu.roll(acc, 32, 1)
                if first and i == 0 and w > 0:
                    pos = lax.broadcasted_iota(jnp.int32, (16, 128), 0) & 7
                    acc = jnp.where(pos >= w, acc, -1e30)
                st["ls"].append(acc)
                st["m"] = acc if w == 0 else jnp.maximum(st["m"], acc)
            return _u(st["m"][0:8])

        def exps(rel):
            m = st["m"]
            st["ps"] = [jnp.exp2(l - m) for l in st["ls"]]
            st["linv"] = 1.0 / functools.reduce(lambda a, b: a + b, st["ps"])
            return _u(st["linv"][0:8])

        def pvs(ts):
            def f(rel):
                if rel is not None:
                    vb[NT + C["za"], 0, 0:8, :] = rel
                tok = None
                for t in ts:
                    acc = None
                    for w in range(8):
                        pr = st["ps"][w] * win(vb, t, w)
                        acc = pr if acc is None else acc + pr
                    acc = acc * st["linv"]
                    o = _pack2r(acc[0:8], acc[8:16])
                    ob[0, 8 * i:8 * i + 8, 128 * t:128 * t + 128] = o
                    tok = o if tok is None else tok | o
                return tok
            return f
        return [(scores, WS), (exps, WE), (pvs([0, 1, 2]), WV), (pvs([3, 4]), WV)]

    def attn_consts():
        lane16 = lax.broadcasted_iota(jnp.int32, (16, 128), 1)
        row16 = lax.broadcasted_iota(jnp.int32, (16, 128), 0)
        grp8 = lax.broadcasted_iota(jnp.int32, (8, 128), 1) // 32
        row32 = lax.broadcasted_iota(jnp.int32, (32, 128), 0)
        lane32 = lax.broadcasted_iota(jnp.int32, (32, 128), 1)
        tri = row32 <= (lane32 & 31)
        mbot = (jnp.where(2 * row16 <= (lane16 & 31), jnp.uint32(0xFFFF), jnp.uint32(0)) |
                jnp.where(2 * row16 + 1 <= (lane16 & 31), jnp.uint32(HI), jnp.uint32(0)))
        return dict(za=z_ref[0], zb=z_ref[1], lane16=lane16, grp8=grp8, odd=(grp8 & 1) == 1, hi=grp8 >= 2,
                    tri=tri, mbot=mbot, mtop=~mbot,
                    never=lax.broadcasted_iota(jnp.int32, (8, 128), 1) < z_ref[2],
                    row8=lax.broadcasted_iota(jnp.int32, (8, 128), 0),
                    zero16=jnp.zeros((16, 128), u32))

    def qk_rows(Q, r):
        return 288 - 32 * max(0, Q.cmin - r)

    def qk_r(Q, g, r, ties, C):
        lane16, zero = C["lane16"], C["zero16"]
        q0 = Q.at(TB // 2, 16 * r)
        ws = []
        for j in range(4):
            f0 = DH * (4 * g + j)
            t, lo = f0 // 128, f0 % 128
            qt = q_ref[t, pl.ds(q0, 16), :]
            if lo + DH <= 128:
                w = jnp.where((lane16 >= lo) & (lane16 < lo + DH), qt, zero)
            else:
                qt1 = q_ref[t + 1, pl.ds(q0, 16), :]
                w = jnp.where(lane16 >= lo, qt, jnp.where(lane16 < lo + DH - 128, qt1, zero))
            ws.append(w)
        wq = _b(_cat([ws[(gm - r) % 4] for gm in range(4)]))
        kmin = max(0, Q.cmin - r)
        n = qk_rows(Q, r)
        s = lax.dot_general(tied(km_ref[g, pl.ds(Q.at(TB // 2, 16 * (r + kmin) - 128), n // 2), :], ties, C), wq,
                            NTDIMS, preferred_element_type=f32)
        sb = sbs[g % 2]
        if kmin == 0:
            mrg = jnp.where(C["tri"], s[n - 32:n], s[0:32])
            mid = s[32:n - 32]
        else:
            mrg = jnp.where(C["tri"], s[n - 32:n], -1e30)
            mid = s[0:n - 32]
        m = jnp.max(mrg, axis=0, keepdims=True)
        if mid.shape[0]:
            sb[r + C['za'], 224 - mid.shape[0]:224, :] = mid
            m = jnp.maximum(jnp.max(mid, axis=0, keepdims=True), m)
        sb[r + C['za'], 224:256, :] = mrg
        return s, m

    def softmax_pieces(Q, g, ms, C):
        zero8 = C["zero16"][0:8]
        sb, tb = sbs[g % 2], tbs[g % 2]
        pw = {}

        mg = {}

        def chunk(r, k, hf):
            o = 32 * k + 16 * hf
            src = sb.at[r + C['zb']]
            if r not in mg:
                mg[r] = ms[r] if mg["rel"] is None else jnp.where(C["never"], mg["rel"], ms[r])
            a = jnp.exp2(src[pl.ds(o, 8, stride=2), :] - mg[r])
            b = jnp.exp2(src[pl.ds(o + 1, 8, stride=2), :] - mg[r])
            return _pack2(a, b)

        def col(c, hf):
            hs = slice(8 * hf, 8 * hf + 8)
            X = [None] * 4
            for r in range(4):
                k = c - r
                if k == 0:
                    pw[r, hf] = chunk(r, 7, hf)
                    X[r] = pw[r, hf] & C["mtop"][hs]
                elif k == 8:
                    X[r] = (pw[r, hf] & C["mbot"][hs]) if (r, hf) in pw else chunk(r, 7, hf)
                elif 0 < k < 8:
                    X[r] = chunk(r, k - 1, hf)
            nz = [r for r in range(4) if X[r] is not None]
            if len(nz) == 1:
                r = nz[0]
                T = [jnp.where(C["grp8"] == (j + r) % 4, X[r], zero8) for j in range(4)]
            else:
                def sel(mask, a, b):
                    if a is None and b is None:
                        return None
                    return jnp.where(mask, zero8 if a is None else a, zero8 if b is None else b)
                U = [sel(C["odd"], X[(p + 1) % 4], X[p]) for p in range(4)]
                Tp = [sel(C["hi"], U[(p + 2) % 4], U[p]) for p in range(4)]
                T = [zero8 if Tp[(-j) % 4] is None else Tp[(-j) % 4] for j in range(4)]
            for j in range(4):
                tb[j + C['za'], 16 * c + 8 * hf:16 * c + 8 * hf + 8, :] = T[j]
            return T[0]

        def piece(cs):
            def f(rel):
                mg.clear()
                mg["rel"] = rel
                return functools.reduce(lambda a, b: a | b, [col(c, hf) for c, hf in cs])
            return f
        grps = [[x for x in cs if x[0] >= Q.cmin] for cs in SM_GROUPS]
        return [(piece(cs), WM) for cs in grps if cs]

    def pv_j(Q, g, j, C):
        h = 4 * g + j
        off = (DH * h) % 16
        base = DH * h - off
        r1 = (off + DH) % 32
        acc = None
        for t in range(Q.cmin // 4, 3):
            v = vt_ref[Q.at(1, t - 1), base // 2:base // 2 + 16, :]
            halves = [v[0:8], v[8:16]]
            hsel = (r1 // 2) // 8
            halves[hsel] = jnp.where(C["row8"] == (r1 // 2) % 8, jnp.uint32(ONE2), halves[hsel])
            vw = _b(_cat(halves))
            tt = _b(tbs[g % 2][j + C['zb'], 64 * t:64 * t + 64, :])
            d = jnp.dot(vw, tt, preferred_element_type=f32)
            acc = d if acc is None else acc + d
        linv = 1.0 / acc[r1:r1 + 1, :]
        lo8 = (off // 8) * 8
        o = acc[lo8:lo8 + 24, :] * linv
        if j:
            o = pltpu.roll(o, 128 - 32 * j, 1)
        ot_ref[DH * h:DH * h + DH, :] = o[off - lo8:off - lo8 + DH, :]
        return _u(o[0:8]) | _u(o[8:16]) | _u(o[16:24])

    def section(stages, load_m, store_m):
        C = attn_consts()
        clock = [0, 0, 0, 0]
        reg = []

        def place(rows):
            m = clock.index(min(clock))
            s = clock[m]
            clock[m] += rows
            return s

        def token(tm):
            best = None
            for lo, rows, res in reg:
                if lo <= tm:
                    r = min((tm - lo) // 8, rows // 8 - 1)
                    if best is None or lo + 8 * r >= best[0]:
                        best = (lo + 8 * r, res, r)
            return None if best is None else best[1][8 * best[2]:8 * best[2] + 8]

        ms = [m_ref[r, 0:1, :] for r in range(4)] if load_m else None
        last_qk = max(i for i, sp in enumerate(stages) if sp.get("qk"))
        for si, sp in enumerate(stages):
            for f in sp.get("pre", []):
                f()
            fl = [f for u in sp.get("fl", []) for f in u]
            P = softmax_pieces(sp["sm"][0], sp["sm"][1], ms, C) if sp.get("sm") else []
            B = [pc for a in sp.get("B", []) for pc in battn_pieces(*a, C)]
            X = sp.get("X", [])
            items = [((ip + 1) / len(P), 0, pc) for ip, pc in enumerate(P)]
            bf = BF if len(B) == 4 else BF2
            if P:
                items += [((int(bf[ib] * len(P)) + 1) / len(P), 1, pc) for ib, pc in enumerate(B)]
                items += [((int(XF * (ix + 1) / len(X) * len(P)) + 1) / len(P), 2, pc) for ix, pc in enumerate(X)]
            else:
                items += [(bf[ib], 1, pc) for ib, pc in enumerate(B)]
                items += [((ix + 1) / len(X), 2, pc) for ix, pc in enumerate(X)]
            items = sorted(items, key=lambda z: z[:2])
            seq = [z[2] for z in items]
            tbeg = min(clock)
            passes = []
            if sp.get("qk"):
                passes += [("q", r, place(qk_rows(sp["qk"][0], r)), qk_rows(sp["qk"][0], r)) for r in range(4)]
            if sp.get("pv"):
                passes += [("p", j, [place(32) for _ in range(sp["pv"][0].cmin // 4, 3)][0], 0) for j in range(4)]
            passes += [("f", u, place(128), 128) for u in range(len(fl))]
            tend = min(clock)
            slots = {}
            lastp = 0
            dl = []
            for s, pc in enumerate(seq):
                tm = tbeg + (s + 1) * (tend - tbeg) // len(seq) - TIE_OFF
                cand = [ip for ip, (kd, _, t0, rows) in enumerate(passes)
                        if ip >= lastp and rows and t0 <= tm < t0 + rows]
                if not cand:
                    cand = [ip for ip, (kd, _, t0, rows) in enumerate(passes)
                            if ip >= lastp and rows and t0 > tm][:1]
                if not cand:
                    cand = [len(passes) - 1]
                ip = cand[0]
                lastp = ip
                t0, rows = passes[ip][2], passes[ip][3]
                r8 = min(max(tm - t0, 0) // 16, rows // 16 - 1)
                while any(x[1] == r8 for x in slots.get(ip, [])) and r8 < rows // 16 - 1:
                    r8 += 1
                slots.setdefault(ip, []).append((s, r8))
                dl.append(t0 + 16 * r8)
            ms_n = []
            pvt = []
            for ip, (kd, idx, t0, rows) in enumerate(passes):
                if ip == len(passes) - HOOK:
                    for f in sp.get("hook", []):
                        f()
                ties = []
                for s, r8 in slots.get(ip, []):
                    if seq[s] is None:
                        continue
                    ties.append((r8, seq[s][0](token(dl[s] - seq[s][1]))))
                if kd == "f" and pvt and (t0 >= pvt[0][0] + PVD or ip == len(passes) - 1):
                    free = [r8 for r8 in range(8) if all(x[0] != r8 for x in ties)]
                    ties.append((free[0], functools.reduce(lambda a, b: a | b, [x[1] for x in pvt])))
                    pvt = []
                if kd == "q":
                    sres, m = qk_r(sp["qk"][0], sp["qk"][1], idx, ties, C)
                    ms_n.append(m)
                    reg.append((t0 + POP_LAT, rows, sres))
                    if si == last_qk and store_m:
                        m_ref[idx] = jnp.broadcast_to(m, (8, 128))
                elif kd == "p":
                    pvt.append((t0, pv_j(sp["pv"][0], sp["pv"][1], idx, C)))
                    if idx == 3 and sp["pv"][2] is not None:
                        oa_transpose(*sp["pv"][2:])
                else:
                    reg.append((t0 + POP_LAT, rows, fl[idx](ties, C)))
            if sp.get("qk"):
                ms = ms_n
            for f in sp.get("post", []):
                f()

    def attn_stages(Q, oa_prev, first=False, last=False):
        sts = []
        for g in range(NG):
            sp = dict(sm=(Q, g), fl=[], B=[], X=[], pre=[], post=[], hook=[])
            if not (last and g == NG - 1):
                sp["qk"] = (Q, g + 1) if g + 1 < NG else (Q + 1, 0)
            if g > 0:
                sp["pv"] = (Q, g - 1, None)
            elif not first:
                sp["pv"] = (Q + (-1), NG - 1, oa_prev)
            sts.append(sp)
        return sts

    def spread(sts, F, cnt):
        assert sum(cnt) == len(F), (sum(cnt), len(F))
        k = 0
        for sp, c in zip(sts, cnt):
            sp["fl"] += F[k:k + c]
            k += c

    def U_qk(Q, ns):
        return [unit(qk_pass, Q, n) for n in ns]

    def U_v(Q):
        return [unit(v_pass, Q, n) for n in range(NT)]

    def U_pb(Q, pn, ns=range(15)):
        return [unit(pb_pass, Q, pn, n) for n in ns]

    def now(pcs):
        return lambda: [pc[0](None) for pc in pcs]

    Z = [Blk(None, b) for b in range(NB)]
    xmb = [[xm_piece(Z[b], i) for i in range(4)] for b in range(4)]
    gps = [g_piece(Z[b], i) for b in range(4) for i in range(4)]
    pre = []
    for n in range(7):
        pre.append(dict(fl=[u for b in range(4) for u in U_qk(Z[b], WORD[n:n + 1])], pre=[], X=gps[3 * n - 3:3 * n] if n else []))
    pre[0]["pre"] = [c_x.wait, cp_wb(1).start, cp_wb(2).start, now([p for b in range(4) for p in xmb[b]]), cw[0].wait,
                     c_wv.start]
    pre[1]["pre"] = [c_gw.wait, cw[1].wait, cw[2].wait] + [cp_woa(n).start for n in range(NT)] + [c_wob.start]
    pre[3]["pre"] = [cw[n].wait for n in range(3, 7)] + [c_xl.start]
    def st(fl, **kw):
        d = dict(fl=fl, pre=[], X=[], B=[])
        d.update(kw)
        return d

    pb = {(b, p): U_pb(Z[b], (2, 1, 0)[b], range(5 * p, 5 * p + 5)) for b in range(3) for p in range(3)}
    pwb = [[prep_wb(p, c) for c in range(NT)] for p in range(3)]
    BB = [(2, obs[0], True, i) for i in range(NG)] + [(1, obs[1], False, i) for i in range(NG)]
    pre.append(st(U_qk(Z[0], WORD[7:10]) + U_qk(Z[1], WORD[7:10]), pre=[cw[n].wait for n in range(7, 10)] + [cp_wb(0).wait],
                  X=[None] + pwb[0][0:2]))
    pre.append(st(U_qk(Z[2], WORD[7:10]) + U_qk(Z[3], WORD[7:10]), X=pwb[0][2:5] + [None]))
    pre.append(st(pb[0, 0]))
    pre.append(st(pb[1, 0][:PB1]))
    pre.append(st(pb[1, 0][PB1:] + pb[2, 0], pre=[cp_wb(1).wait, cp_wb(2).wait], X=[None] * XN + pwb[1]))
    pre.append(st(pb[0, 1], X=pwb[2] + [None]))
    pre.append(st(pb[0, 2] + pb[1, 1][:PB2], pre=[c_wv.wait], X=[None] * XN + [prep_wv(c) for c in range(NT)]))
    v0 = U_v(Z[0])
    ee = [st(v0[0:2], B=[BB[0]]), st(v0[2:5], qk=(Z[0], 0), B=[BB[1]])]
    b0 = attn_stages(Z[0], None, first=True)
    b1 = attn_stages(Z[1], oas[0])
    spread(b0 + b1, pb[1, 1][PB2:] + pb[1, 2] + U_v(Z[1]) + pb[2, 1] + pb[2, 2] + U_v(Z[2]) + U_o(Z[0], oas[0], obs[0]), B01CNT)
    for i, s in enumerate(B1POS):
        (b0 + b1)[s]["B"].append(BB[2 + i])
    (b0 + b1)[B1POS[6]]["pre"].append(lambda: halo_copy(1, 2))
    b0[P7]["pre"] += [cp_woa(n).wait for n in range(NT)] + [c_wob.wait]
    for c in range(NT):
        (b0 + b1)[P7 + 1 + c]["X"].append(prep_wob(c))
    section(pre + ee + b0 + b1, False, True)
    cp_o(0, TB, 6).start()
    c_xl.wait()

    def mid_block(Q, par):
        sts = attn_stages(Q, oas[0])
        sts[0]["pre"].append(lambda: halo_copy(par))
        src = dict(b=U_pb(Q + 1, 1 - par), o=U_o(Q + (-1), oas[0], obs[1 - par]), v=U_v(Q + 1),
                   q=U_qk(Q + 2, range(5)), k=U_qk(Q + 2, range(5, 10)))
        for sp, w in zip(sts, ORD.split()):
            sp["fl"] += [src[ch].pop(0) for ch in w]
        assert not any(src.values())
        for g in range(NG):
            sts[g]["B"] = [(par, obs[par], False, g)]
        for i in range(4):
            sts[i // 2]["X"].append(xm_piece(Q + 2, i))
            sts[4 + i]["X"].append(g_piece(Q + 2, i))
        return sts

    def p2(i, carry):
        Q = Blk(i, 2)
        section(mid_block(Q, 0) + mid_block(Q + 1, 1), True, True)
        cp_o(Q.at(TB, -TB), 2 * TB, i).start()
        return carry

    lax.fori_loop(0, 6, p2, 0)

    b14 = attn_stages(Z[14], oas[1])
    b14[0]["pre"].append(lambda: halo_copy(0))
    spread(b14, U_pb(Z[15], 1) + U_v(Z[15]), [2, 3, 2, 3, 2, 3, 2, 3])
    b15 = attn_stages(Z[15], oas[0], last=True)
    b15[0]["pre"].append(lambda: halo_copy(1))
    spread(b15, U_o(Z[13], oas[1], obs[1]) + U_o(Z[14], oas[0], obs[0]), [2, 2, 2, 2, 2, 4, 2, 4])
    b15[4]["post"].append(cp_o(13 * TB, TB, 7).start)
    for g in range(NG):
        b14[g]["B"] = [(0, obs[0], False, g)]
        b15[g]["B"] = [(1, obs[2], False, g)]
    b15[7]["pv"] = (Z[15], NG - 2, oas[1], range(NT - 1))
    early = []
    for n in range(NT):
        s_ = {}
        early.append([functools.partial(ob_pass, obs[2], n, k, s_) for k in range(NT)] +
                     [functools.partial(oa_early, Z[15], oas[1], n, k, s_) for k in range(NT - 1)])
    late = [[functools.partial(oa_late, Z[15], oas[1], n) for n in range(NT)]]
    tail = [dict(pre=[cp_o(14 * TB, TB, 8).start], pv=(Z[15], NG - 1, oas[1], [NT - 1]), fl=early + late)]
    section(b14 + b15 + tail, True, False)
    cp_o(15 * TB, TB, 9).start()
    cp_o(0, TB, 6).wait()
    for i in range(6):
        cp_o((2 * i + 1) * TB, 2 * TB, i).wait()
    for k in range(3):
        cp_o((13 + k) * TB, TB, 7 + k).wait()


@jax.jit
def pallas_gated_mix__sliding_block__sliding_local_dilated__prompt_kernel(A_x, A_wqkv, A_wo, B_x, B_wqkv, B_wo, gate_w):
    x = A_x.reshape(S, D)
    bbuf = [pltpu.VMEM((NT, TB, 128), f32), pltpu.VMEM((NT + 1, 2, HALO + TB // 2, 128), f32),
            pltpu.VMEM((NT + 1, 2, HALO + TB // 2, 128), f32)]
    out = pl.pallas_call(
        kernel,
        out_shape=jax.ShapeDtypeStruct((S, D), bf16),
        in_specs=[pl.BlockSpec(memory_space=pl.ANY)] * 6,
        out_specs=pl.BlockSpec(memory_space=pl.ANY),
        scratch_shapes=[
            pltpu.VMEM((S, D), bf16),
            pltpu.VMEM((2 * NT, D, 128), bf16),
            pltpu.VMEM((D, D), bf16),
            pltpu.VMEM((NT, D, 128), bf16),
            pltpu.VMEM((3, D, D), bf16),
            pltpu.VMEM((D, D), bf16),
            pltpu.VMEM((D,), bf16),
            pltpu.VMEM((S, D), bf16),
            pltpu.SemaphoreType.DMA((5,)),
            pltpu.VMEM((3 * NT, D // 2, 128), u32),
            pltpu.VMEM((NT, S // 2, 128), u32),
            pltpu.VMEM((NT, S // 2, 128), u32),
            pltpu.VMEM((S, 128), f32),
            pltpu.VMEM((NT, S // 2, 128), u32),
            pltpu.VMEM((NG, S // 2, 128), u32),
            pltpu.VMEM((NB + 1, D // 2, 128), u32),
            pltpu.VMEM((D // 2, D), u32),
            pltpu.VMEM((3 * D // 2, D), u32),
            pltpu.VMEM((D // 2, D), u32),
            pltpu.VMEM((NT, D // 2, 128), u32),
        ] + bbuf + bbuf + bbuf + [
            pltpu.VMEM((D, 128), f32),
            pltpu.VMEM((TB // 2, D), u32),
            pltpu.VMEM((TB // 2, D), u32),
            pltpu.VMEM((1, TB // 2, D), u32),
            pltpu.VMEM((1, TB // 2, D), u32),
            pltpu.VMEM((1, TB // 2, D), u32),
            pltpu.VMEM((4, 256, 128), f32),
            pltpu.VMEM((4, 256, 128), f32),
            pltpu.VMEM((4, 192, 128), u32),
            pltpu.VMEM((4, 192, 128), u32),
            pltpu.VMEM((4, 8, 128), f32),
            pltpu.SMEM((3,), jnp.int32),
        ],
        compiler_params=pltpu.CompilerParams(vmem_limit_bytes=100 * 1024 * 1024),
    )(x, A_wqkv, A_wo, B_wqkv, B_wo, gate_w)
    return out.reshape(1, S, D)
```

```python
import functools
import math

import jax
import jax.numpy as jnp
from jax import lax
from jax.experimental import pallas as pl
from jax.experimental.pallas import tpu as pltpu

S, D, H, DH = 2048, 640, 32, 20
TB = 128
NB = S // TB
NT = D // 128
NG = 8
QSCALE = DH ** -0.5 * math.log2(math.e)
ONE2 = 0x3F803F80
HI = 0xFFFF0000
TIE_OFF = 16
POP_LAT = 130
SMT = 4


def sm_groups(smt):
    grps, acc, cur = [], 0, []
    for c in range(12):
        for hf in range(2):
            cur.append((c, hf))
            acc += sum(1 for r in range(4) if 0 <= c - r < 8)
            if acc >= smt:
                grps.append(cur)
                acc, cur = 0, []
    grps[-1] = grps[-1] + cur
    return grps


BF = [0.5, 0.6, 0.72, 0.99]
BF2 = [0.25, 0.35, 0.5, 0.6, 0.6, 0.7, 0.85, 0.99]
XF = 0.3
WS = 350
WE = 100000
WV = 200
WP = 100000
HOOK = 1
B01CNT = [2, 4, 3, 3, 3, 3, 2, 2, 2, 2, 2, 2, 2, 2, 2, 2]
B1POS = [0, 1, 2, 3, 4, 5, 6, 7, 8, 9, 10, 12, 13, 15]
P7 = 4
PB1 = 4
PB2 = 2
XN = 1
WX = 600
PVD = 750
WM = 200
ORD = "obbbb bbbbo kvoob kboov qbook qkbqb qvovo qkvbb"
HALO = 8
BPI = 3
ORD3 = "bbbbb bbboo kooov kvobb ovqvo koovb qbkqb qkqbb"
SP = {8: {'WS': 575, 'PL': 138}, 11: {'BF': [0.5, 0.6, 0.6, 0.99], 'XF': 0.7}, 18: {'WV': 350, 'BF': [0.38, 0.54, 0.6, 0.99], 'PVD': 600, 'XF': 0.6, 'WM': 200, 'TO': 32}, 21: {'WS': 525, 'TO': 40, 'BF': [0.5, 0.54, 0.66, 0.99], 'PL': 146, 'PVD': 400, 'SMT': 6, 'QO': 0}, 24: {'TO': 56, 'WM': 225, 'WV': 350, 'QO': 1, 'XF': 0.8, 'WS': 500, 'BF': [0.5, 0.54, 0.6, 0.93]}, 27: {'TO': 72, 'SMT': 6, 'PVD': 450, 'BF': [0.5, 0.54, 0.66, 0.99], 'WV': 275}, 30: {'WV': 175, 'TO': 24, 'WM': 250, 'BF': [0.5, 0.54, 0.66, 0.99], 'XF': 0.9}, 12: {'TO': 8, 'WV': 225, 'WS': 450, 'PVD': 600, 'WM': 100, 'BF': [0.5, 0.54, 0.72, 0.99]}, 29: {'WS': 650, 'BF': [0.5, 0.6, 0.66, 0.99], 'WV': 250, 'PL': 162}, 28: {'PL': 130, 'WV': 125, 'BF': [0.5, 0.54, 0.72, 0.99]}, 25: {'WM': 100, 'QO': 0, 'WS': 475}, 7: {'XF': 0.6, 'PL': 162, 'WM': 150}, 10: {'TO': 8, 'WS': 575}, 13: {'WM': 175, 'SMT': 3, 'TO': 32}, 17: {'WM': 150, 'BF': [0.5, 0.54, 0.6, 0.93]}, 20: {'PVD': 900, 'QO': 1, 'PL': 130}, 15: {'WS': 525, 'BF': [0.48, 0.5, 0.54, 0.99]}, 9: {'PVD': 600, 'WM': 100, 'TO': 32}, 16: {'PVD': 900}, 19: {'BF': [0.5, 0.54, 0.72, 0.99]}, 22: {'SMT': 6}, 31: {'PL': 162, 'WV': 250}, 23: {'WM': 175, 'TO': 24, 'PL': 130}, 26: {'WS': 500, 'WV': 175}}
SL = {2: {'BF': [0.38, 0.6, 0.72, 0.99], 'WV': 300, 'WM': 325}, 7: {'TO': 40, 'WV': 175, 'BF': [0.5, 0.54, 0.66, 0.93], 'XF': 0.1}, 10: {'BF': [0.48, 0.5, 0.78, 0.93], 'XF': 0.4, 'QO': 2, 'WM': 175, 'WS': 325, 'WV': 300}, 13: {'WS': 325, 'WM': 325, 'BF': [0.44, 0.54, 0.72, 0.93], 'WV': 225, 'SMT': 5}, 1: {'BF': [0.38, 0.54, 0.72, 0.93], 'PL': 122, 'XF': 0.5, 'WS': 350, 'SMT': 6}, 6: {'BF': [0.5, 0.6, 0.72, 0.81], 'QO': 1, 'XF': 0.95}, 9: {'WV': 150, 'XF': 0.6, 'WM': 300, 'SMT': 4, 'PL': 130, 'TO': 48}, 12: {'XF': 0.4, 'WM': 375, 'TO': 24, 'WS': 450, 'BF': [0.5, 0.6, 0.72, 0.99]}, 8: {'PL': 106, 'TO': 64, 'PVD': 1000, 'QO': 1, 'BF': [0.48, 0.5, 0.72, 0.93], 'WM': 300, 'XF': 0.95, 'WV': 250}, 5: {'TO': 64, 'PL': 106, 'BF': [0.5, 0.6, 0.84, 0.93], 'WV': 300}, 15: {'WV': 125, 'WS': 450, 'TO': 16, 'SMT': 3, 'XF': 0.95}, 18: {'WS': 325, 'TO': 48, 'QO': 0, 'XF': 0.8, 'BF': [0.56, 0.6, 0.72, 0.93], 'WM': 375, 'WV': 300}, 21: {'WV': 325, 'QO': 2}, 3: {'WM': 325}, 11: {'PVD': 700, 'WM': 400, 'BF': [0.44, 0.6, 0.72, 0.93]}, 14: {'XF': 0.1, 'WS': 500, 'WM': 125, 'TO': 64, 'QO': 2, 'PL': 106}, 17: {'WV': 100, 'BF': [0.5, 0.6, 0.72, 0.87], 'WM': 325, 'XF': 0.8, 'PL': 122}, 20: {'TO': 24, 'PVD': 700, 'PL': 98, 'XF': 0.6, 'WS': 375, 'WV': 225, 'WM': 250, 'QO': 2}, 23: {'XF': 0.5, 'WM': 325, 'SMT': 3, 'TO': 64, 'WS': 450, 'QO': 2}, 22: {'WM': 325, 'WS': 450, 'BF': [0.5, 0.6, 0.78, 0.93], 'PVD': 700}, 0: {'PVD': 550, 'BF': [0.5, 0.6, 0.72, 0.99], 'TO': 48, 'LEAD': 5}, 4: {'QO': 0, 'WV': 225, 'WM': 325, 'WS': 375}, 16: {'WS': 400, 'BF': [0.38, 0.6, 0.72, 0.93], 'XF': 0.6, 'WM': 175}, 19: {'WM': 125, 'PL': 98, 'QO': 1, 'WS': 375, 'WV': 300, 'PVD': 700}}
SE = {0: {'TO': 0, 'WM': 250, 'BF': [0.3, 0.51, 0.65, 0.9], 'WV': 200, 'PVD': 450, 'WS': 675, 'QO': 2}, 3: {'WS': 650, 'TO': 8, 'BF': [0.3, 0.45, 0.65, 0.99], 'SMT': 3}, 6: {'PVD': 600, 'WM': 200, 'TO': 32}, 9: {'QO': 2, 'WV': 275}, 12: {'PL': 138, 'SMT': 5, 'WS': 550, 'TO': 8}, 15: {'BF': [0.42, 0.45, 0.65, 0.9], 'PL': 146, 'SMT': 3, 'WV': 350, 'WS': 525, 'XF': 0.8, 'PVD': 450}, 2: {'PL': 162, 'WV': 275, 'BF': [0.3, 0.45, 0.65, 0.96]}, 5: {'WV': 175, 'BF': [0.3, 0.33, 0.65, 0.9]}, 8: {'WM': 225, 'BF': [0.3, 0.53, 0.57, 0.9]}, 11: {'WV': 275, 'XF': 0.3, 'TO': 48, 'QO': 0}, 14: {'WS': 425, 'XF': 0.2}, 10: {'TO': 48, 'PL': 138, 'SMT': 3, 'WV': 250}, 1: {'PVD': 450, 'XF': 0.4, 'WS': 450, 'BF': [0.3, 0.51, 0.65, 0.9], 'WV': 325}, 4: {'PVD': 600, 'BF': [0.3, 0.33, 0.65, 0.9], 'XF': 0.7}, 7: {'PL': 138, 'TO': 8, 'PVD': 450}, 13: {'WS': 425, 'BF': [0.3, 0.45, 0.65, 0.78]}, 16: {'WS': 575, 'BF': [0.3, 0.33, 0.77, 0.9], 'WM': 325, 'WV': 350, 'TO': 0}}
LS = 2
ORD2 = "bobbb bbbbo kokob ovovo qbobk qoqqb kvkov qbvbb"
EORD = "bb bbb bb bbb bb bv bvb vv voo oo oo op ooo ppp pp pppp"
KD = dict(WS=WS, WV=WV, WM=WM, BF=BF, TO=TIE_OFF, PVD=PVD, XF=XF, SMT=SMT, PL=POP_LAT, QO=0, LEAD=0, LSP=1, LSN=1, EX=0)
KL = dict(KD, **{'WS': 350, 'WV': 200, 'WM': 225, 'BF': [0.5, 0.6, 0.72, 0.93], 'TO': 32, 'PVD': 850, 'XF': 0.3, 'SMT': 4, 'PL': 114})
KL.update(dict(LSP=4,EX=1))
KP = dict(KD, **{'WS': 500, 'WV': 275, 'WM': 200, 'BF': [0.5, 0.54, 0.6, 0.99], 'TO': 16, 'PVD': 550, 'XF': 0.7, 'SMT': 4, 'PL': 146, 'QO': 2, 'LEAD': 0})
KE = dict(KD, **{'WS': 550, 'WV': 300, 'WM': 300, 'BF': [0.3, 0.45, 0.65, 0.9], 'TO': 16, 'PVD': 750, 'XF': 0.6, 'SMT': 4, 'PL': 130, 'QO': 2})
XA = 2
WA = 2
WB = 3
HB = [11]
NTDIMS = (((1,), (1,)), ((), ()))

f32 = jnp.float32
bf16 = jnp.bfloat16
u32 = jnp.uint32


def _u(x):
    return pltpu.bitcast(x, u32)


def _b(x):
    return pltpu.bitcast(x, bf16)


def _f(x):
    return pltpu.bitcast(x, f32)


def _pack2(a, b):
    return (_u(a) >> 16) | (_u(b) & jnp.uint32(HI))


def _pack2r(a, b):
    h = jnp.uint32(0x8000)
    return ((_u(a) + h) >> 16) | ((_u(b) + h) & jnp.uint32(HI))


def _cat(xs):
    return jnp.concatenate(xs, axis=0)


class Blk:
    def __init__(self, i, off, cache=None):
        self.i, self.off, self.cache = i, off, ({} if cache is None else cache)

    def __add__(self, k):
        return Blk(self.i, self.off + k, self.cache)

    def at(self, per, extra=0):
        c = self.off * per + extra
        if self.i is None:
            return c
        if per not in self.cache:
            self.cache[per] = self.i * (BPI * per)
        al = math.gcd(BPI * per, c)
        v = self.cache[per] + c
        return pl.multiple_of(v, al) if al > 1 else v

    @property
    def cmin(self):
        return max(0, 8 - 4 * self.off) if self.i is None else 0


def kernel(x_hbm, wa_hbm, woa_hbm, wb_hbm, wob_hbm, gw_hbm, o_hbm,
           x_ref, wqk_ref, wv_ref, woa_ref, wb_ref, wob_ref, gw_ref, o_ref, sem,
           wu_ref, xu_ref, xm_ref, g_ref, q_ref, km_ref, vt_ref, wvt_ref, wbpt_ref, wobp_ref, tmp_ref,
           qb0, kb0, vb0, qb1, kb1, vb1, qb2, kb2, vb2, ot_ref, oa0, oa1, ob0, ob1, ob2, s0, s1, t0_, t1_, m_ref, z_ref):
    sbs, tbs = (s0, s1), (t0_, t1_)
    qbs, kbs, vbs, obs, oas = (qb0, qb1, qb2), (kb0, kb1, kb2), (vb0, vb1, vb2), (ob0, ob1, ob2), (oa0, oa1)

    def cp_x(r0, n, k):
        return pltpu.make_async_copy(x_hbm.at[pl.ds(r0, n), :], x_ref.at[pl.ds(r0, n), :], sem.at[k])

    def cp_w(n0, n1, k):
        cs = pl.ds(128 * n0, 128 * (n1 - n0))
        return pltpu.make_async_copy(wa_hbm.at[:, cs], wqk_ref.at[:, cs], sem.at[k])

    def cp_wb(p):
        return pltpu.make_async_copy(wb_hbm.at[:, pl.ds(D * p, D)], wb_ref.at[p], sem.at[(4, 0, 0)[p]])

    def cp_o(r0, n, k):
        return pltpu.make_async_copy(o_ref.at[pl.ds(r0, n), :], o_hbm.at[pl.ds(r0, n), :], sem.at[4])

    c_x = cp_x(0, XA * TB, 0)
    c_x2 = cp_x(XA * TB, (4 - XA) * TB, 2)
    c_xl = cp_x(4 * TB, S - 4 * TB, 3)
    c_gw = pltpu.make_async_copy(gw_hbm, gw_ref, sem.at[2])
    c_wv = pltpu.make_async_copy(wa_hbm.at[:, pl.ds(2 * D, D)], wv_ref, sem.at[1])
    c_wob = pltpu.make_async_copy(wob_hbm, wob_ref, sem.at[2])
    c_woa = pltpu.make_async_copy(woa_hbm, woa_ref, sem.at[2])
    WORD = list(range(10))
    cw = [cp_w(0, WA, 1), cp_w(WA, WB, 2), cp_w(WB, 7, 3), cp_w(7, 10, 4)]
    for c in [c_x, cw[0], c_gw, c_x2, cw[1], cw[2], cp_wb(0), cw[3]]:
        c.start()

    z_ref[0] = 0
    z_ref[1] = 0
    z_ref[2] = 0
    kb2[0:NT, :, 0:HALO, :] = jnp.zeros((NT, 2, HALO, 128), f32)
    vb2[0:NT, :, 0:HALO, :] = jnp.zeros((NT, 2, HALO, 128), f32)
    vt_ref[0, D // 2 - 48:D // 2, :] = jnp.zeros((48, 128), u32)
    t1_[:, 0:64, :] = jnp.zeros((4, 64, 128), u32)

    def deint(src, dst, doff, cs):
        tok = None
        for e in range(DH // 2):
            rows = src[pl.ds(e, H, stride=DH // 2), :]
            a = _cat([rows[0:8], rows[16:24]])
            b = _cat([rows[8:16], rows[24:32]])
            lo = (a & jnp.uint32(0xFFFF)) | (b << 16)
            hi = (a >> 16) | (b & jnp.uint32(HI))
            dst[doff + 32 * e:doff + 32 * e + 16, cs] = lo
            dst[doff + 32 * e + 16:doff + 32 * e + 32, cs] = hi
            tok = hi[8:16] if tok is None else tok | hi[8:16]
        return tok

    def gated(w, rel):
        if rel is None:
            return w
        never = lax.broadcasted_iota(jnp.int32, (8, 128), 1) < z_ref[2]
        z = jnp.where(never, _u(rel), jnp.uint32(0))
        return w | jnp.tile(z, (w.shape[0] // 8, w.shape[1] // 128))

    def prep_wb(p, c):
        def f(rel):
            cs = slice(128 * c, 128 * c + 128)
            tmp_ref[c] = _u(_b(gated(_u(wb_ref[p, cs, :]), rel)).T)
            return deint(tmp_ref.at[c], wbpt_ref, 320 * p, cs)
        return (f, WX)

    def prep_wob(c):
        def f(rel):
            cs = slice(128 * c, 128 * c + 128)
            tmp_ref[c] = gated(_u(wob_ref[:, cs]), rel)
            return deint(tmp_ref.at[c], wobp_ref, 0, cs)
        return (f, WX)

    def prep_wv(c):
        def f(rel):
            cs = slice(128 * c, 128 * c + 128)
            w = _u(_b(gated(_u(wv_ref[cs, :]), rel)).T)
            wvt_ref[:, cs] = w
            return functools.reduce(lambda a, b: a | b, [w[64 * i + 56:64 * i + 64] for i in range(NT)])
        return (f, WX)

    def xm_piece(Q, i):
        def f(rel):
            r0, h0 = Q.at(TB, 32 * i), Q.at(TB // 2, 16 * i)
            xw = _u(x_ref[pl.ds(r0, 32), :])
            tok = None
            for t in range(NT):
                xu_ref[t, pl.ds(h0, 16), :] = xw[:, 128 * t:128 * t + 128]
                src = xu_ref.at[t, pl.ds(h0, 16), :]
                a = src[pl.ds(0, 8, stride=2), :]
                b = src[pl.ds(1, 8, stride=2), :]
                lo = (a & jnp.uint32(0xFFFF)) | (b << 16)
                hi = (a >> 16) | (b & jnp.uint32(HI))
                xm_ref[t, pl.ds(h0, 16), :] = _cat([lo, hi])
                tok = (lo | hi) if tok is None else tok | lo | hi
            return tok
        return (f, WP)

    def g_piece(Q, i):
        def f(rel):
            r0, h0 = Q.at(TB, 32 * i), Q.at(TB // 2, 16 * i)
            gw = gw_ref[...].astype(f32).reshape(1, D)
            z = None
            for t in range(NT):
                xb = _b(xu_ref[t, pl.ds(h0, 16), :]).astype(f32) * gw[:, 128 * t:128 * t + 128]
                z = xb if z is None else z + xb
            z = jnp.sum(z, axis=-1, keepdims=True)
            g = jnp.broadcast_to(jax.nn.sigmoid(z), (32, 128))
            g_ref[pl.ds(r0, 32), :] = g
            return _u(g[0:8]) | _u(g[8:16]) | _u(g[16:24]) | _u(g[24:32])
        return (f, WP)

    def accum(st, key, k, d, C):
        a = st[key] = d if k == 0 else (d + st[key] if C['EX'] else st[key] + d)
        return a, (a if C['EX'] else d)

    def tied(x, ties, C):
        for r8, tok in ties:
            rows = []
            if r8 > 0:
                rows.append(x[:8 * r8])
            rows.append(jnp.where(C["never"], tok, x[8 * r8:8 * r8 + 8]))
            if 8 * r8 + 8 < x.shape[0]:
                rows.append(x[8 * r8 + 8:])
            x = _cat(rows)
        return _b(x)

    def nat(res):
        return _cat([_pack2r(res[32 * i:32 * i + 16], res[32 * i + 16:32 * i + 32]) for i in range(TB // 32)])

    def qk_pass(Q, n, k, st, ties, C):
        h0 = Q.at(TB // 2)
        xb = tied(xm_ref[k, pl.ds(h0, TB // 2), :], ties, C)
        w = wqk_ref[128 * k:128 * k + 128, 128 * n:128 * n + 128] if Q.i is None else _b(wu_ref[n, 64 * k:64 * k + 64, :])
        if Q.i is None and Q.off == 3:
            wu_ref[n, 64 * k:64 * k + 64, :] = _u(w)
        d = jnp.dot(xb, w, preferred_element_type=f32)
        res, d = accum(st, "acc", k, d, C)
        if k == NT - 1:
            if n < NT:
                q_ref[n, pl.ds(h0, TB // 2), :] = nat(res * QSCALE)
            else:
                t = n - NT
                kt = nat(res)
                for g in range(NG):
                    t0, t1, lg = (80 * g) // 128, (80 * g + 79) // 128, (80 * g + 80) % 128
                    if t0 == t1 == t:
                        km_ref[g, pl.ds(h0, TB // 2), :] = kt
                    elif t0 == t:
                        km_ref[g, pl.ds(h0, TB // 2), lg:128] = kt[:, lg:128]
                    elif t1 == t:
                        km_ref[g, pl.ds(h0, TB // 2), 0:lg] = kt[:, 0:lg]
        return d

    def v_pass(Q, n, k, st, ties, C):
        lhs = tied(wvt_ref[64 * n:64 * n + 64, 128 * k:128 * k + 128], ties, C)
        w = _b(xu_ref[k, pl.ds(Q.at(TB // 2), TB // 2), :])
        d = lax.dot_general(lhs, w, NTDIMS, preferred_element_type=f32)
        res, d = accum(st, "acc", k, d, C)
        if k == NT - 1:
            vt_ref[Q.at(1, 1), 64 * n:64 * n + 64, :] = _u(res.astype(bf16))
        return d

    def pb_pass(Q, pn, n, k, st, ties, C):
        xb = tied(xm_ref[k, pl.ds(Q.at(TB // 2), TB // 2), :], ties, C)
        w = _b(wbpt_ref[64 * n:64 * n + 64, 128 * k:128 * k + 128])
        R = TB // C.get('split', 1)
        d = _cat([lax.dot_general(xb[r:r + R], w, NTDIMS, preferred_element_type=f32) for r in range(0, TB, R)])
        res, d = accum(st, "acc", k, d, C)
        if k == NT - 1:
            p, t = n // NT, n % NT
            if p == 0:
                qbs[pn][t] = res * QSCALE
            else:
                dst = (kbs if p == 1 else vbs)[pn]
                for i in range(TB // 32):
                    for e in range(2):
                        dst[t, e, HALO + 16 * i:HALO + 16 * i + 16, :] = res[32 * i + 16 * e:32 * i + 16 * e + 16]
        return d

    def halo_copy(par, src=None):
        for bufs in (kbs, vbs):
            bufs[par][0:NT, :, 0:HALO, :] = bufs[1 - par if src is None else src][0:NT, :, TB // 2:TB // 2 + HALO, :]

    def oa_transpose(oa, ts=range(NT)):
        for t in ts:
            oa[0, :, 128 * t:128 * t + 128] = _u(ot_ref[128 * t:128 * t + 128, :].astype(bf16).T)

    def ob_pass(ob, n, k, st, ties, C):
        d = jnp.dot(tied(ob[C['zb'], :, 128 * k:128 * k + 128], ties, C),
                    _b(wobp_ref[64 * k:64 * k + 64, 128 * n:128 * n + 128]), preferred_element_type=f32)
        _, d = accum(st, "b", k, d, C)
        return d

    def oa_pass(Qo, oa, n, k, st, ties, C):
        if Qo.i is None and Qo.off == 0:
            w = woa_ref[128 * k:128 * k + 128, 128 * n:128 * n + 128]
            wu_ref[10 + n, 64 * k:64 * k + 64, :] = _u(w)
        else:
            w = _b(wu_ref[10 + n, 64 * k:64 * k + 64, :])
        d = jnp.dot(tied(oa[C['zb'] if Qo.i is None else 0, :, 128 * k:128 * k + 128], ties, C), w, preferred_element_type=f32)
        a, d = accum(st, "a", k, d, C)
        if k == NT - 1:
            r0 = Qo.at(TB)
            gate = g_ref[pl.ds(r0, TB), :]
            b = st["b"]
            o_ref[pl.ds(r0, TB), 128 * n:128 * n + 128] = (b + gate * (a - b)).astype(bf16)
        return d

    def oa_early(Qo, oa, n, k, st, ties, C):
        d = jnp.dot(tied(oa[0, :, 128 * k:128 * k + 128], ties, C), _b(wu_ref[10 + n, 64 * k:64 * k + 64, :]),
                    preferred_element_type=f32)
        a, d = accum(st, "a", k, d, C)
        if k == NT - 2:
            b = st["b"]
            qb0[n] = b + g_ref[pl.ds(Qo.at(TB), TB), :] * (a - b)
        return d

    def oa_late(Qo, oa, n, h, nh, ties, C):
        k, R = NT - 1, TB // nh
        r0 = Qo.at(TB, R * h)
        d = jnp.dot(tied(oa[0, R // 2 * h:R // 2 * (h + 1), 128 * k:128 * k + 128], ties, C),
                    _b(wu_ref[10 + n, 64 * k:64 * k + 64, :]), preferred_element_type=f32)
        o_ref[pl.ds(r0, R), 128 * n:128 * n + 128] = (qb0[n, R * h:R * (h + 1), :] + g_ref[pl.ds(r0, R), :] * d).astype(bf16)
        if n == NT - 1:
            cp_o(r0, R, 9).start()
        return d

    def unit(fn, *args):
        st = {}
        return [functools.partial(fn, *args, k, st) for k in range(NT)]

    def U_o(Qo, oa, ob):
        us = []
        for n in range(NT):
            st = {}
            us.append([functools.partial(ob_pass, ob, n, k, st) for k in range(NT)])
            us.append([functools.partial(oa_pass, Qo, oa, n, k, st) for k in range(NT)])
        return us

    def battn_pieces(par, ob, first, i, C):
        qb, kb, vb = qbs[par], kbs[par], vbs[par]
        st = {"ls": []}
        q0 = 32 * (i // 2) + 8 * (i % 2)

        def win(buf, t, w):
            o = HALO + 8 * i - w
            return _cat([buf[t, 0, o:o + 8, :], buf[t, 1, o:o + 8, :]])

        def scores(rel):
            q = [[qb[t, q0:q0 + 8, :], qb[t, q0 + 16:q0 + 24, :]] for t in range(NT)]
            if rel is not None:
                q = [[jnp.where(C["never"], rel, v) for v in vv] for vv in q]
            q = [_cat(vv) for vv in q]
            for w in range(8):
                acc = None
                for t in range(NT):
                    pr = q[t] * win(kb, t, w)
                    acc = pr if acc is None else acc + pr
                acc = acc + pltpu.roll(acc, 64, 1)
                acc = acc + pltpu.roll(acc, 32, 1)
                if first and i == 0 and w > 0:
                    pos = lax.broadcasted_iota(jnp.int32, (16, 128), 0) & 7
                    acc = jnp.where(pos >= w, acc, -1e30)
                st["ls"].append(acc)
                st["m"] = acc if w == 0 else jnp.maximum(st["m"], acc)
            return _u(st["m"][0:8])

        def exps(rel):
            m = st["m"]
            st["ps"] = [jnp.exp2(l - m) for l in st["ls"]]
            st["linv"] = 1.0 / functools.reduce(lambda a, b: a + b, st["ps"])
            return _u(st["linv"][0:8])

        def pvs(ts):
            def f(rel):
                if rel is not None:
                    vb[NT + C["za"], 0, 0:8, :] = rel
                tok = None
                for t in ts:
                    acc = None
                    for w in range(8):
                        pr = st["ps"][w] * win(vb, t, w)
                        acc = pr if acc is None else acc + pr
                    acc = acc * st["linv"]
                    o = _pack2r(acc[0:8], acc[8:16])
                    ob[0, 8 * i:8 * i + 8, 128 * t:128 * t + 128] = o
                    tok = o if tok is None else tok | o
                return tok
            return f
        return [(scores, C['WS']), (exps, WE), (pvs([0, 1, 2]), C['WV']), (pvs([3, 4]), C['WV'])]

    def attn_consts():
        lane16 = lax.broadcasted_iota(jnp.int32, (16, 128), 1)
        row16 = lax.broadcasted_iota(jnp.int32, (16, 128), 0)
        grp8 = lax.broadcasted_iota(jnp.int32, (8, 128), 1) // 32
        row32 = lax.broadcasted_iota(jnp.int32, (32, 128), 0)
        lane32 = lax.broadcasted_iota(jnp.int32, (32, 128), 1)
        tri = row32 <= (lane32 & 31)
        mbot = (jnp.where(2 * row16 <= (lane16 & 31), jnp.uint32(0xFFFF), jnp.uint32(0)) |
                jnp.where(2 * row16 + 1 <= (lane16 & 31), jnp.uint32(HI), jnp.uint32(0)))
        return dict(za=z_ref[0], zb=z_ref[1], lane16=lane16, grp8=grp8, odd=(grp8 & 1) == 1, hi=grp8 >= 2,
                    tri=tri, mbot=mbot, mtop=~mbot,
                    never=lax.broadcasted_iota(jnp.int32, (8, 128), 1) < z_ref[2],
                    row8=lax.broadcasted_iota(jnp.int32, (8, 128), 0),
                    zero16=jnp.zeros((16, 128), u32))

    def qk_rows(Q, r):
        return 288 - 32 * max(0, Q.cmin - r)

    def qk_r(Q, g, r, ties, C):
        lane16, zero = C["lane16"], C["zero16"]
        q0 = Q.at(TB // 2, 16 * r)
        ws = []
        for j in range(4):
            f0 = DH * (4 * g + j)
            t, lo = f0 // 128, f0 % 128
            qt = q_ref[t, pl.ds(q0, 16), :]
            if lo + DH <= 128:
                w = jnp.where((lane16 >= lo) & (lane16 < lo + DH), qt, zero)
            else:
                qt1 = q_ref[t + 1, pl.ds(q0, 16), :]
                w = jnp.where(lane16 >= lo, qt, jnp.where(lane16 < lo + DH - 128, qt1, zero))
            ws.append(w)
        wq = _b(_cat([ws[(gm - r) % 4] for gm in range(4)]))
        kmin = max(0, Q.cmin - r)
        n = qk_rows(Q, r)
        kk = km_ref[g, pl.ds(Q.at(TB // 2, 16 * (r + kmin) - 128), n // 2), :]
        qo = C['QO'] if kmin == 0 else 0
        if qo == 1:
            kk = _cat([kk[16:n // 2 - 16], kk[0:16], kk[n // 2 - 16:]])
        elif qo == 2:
            kk = _cat([kk[0:16], kk[n // 2 - 16:], kk[16:n // 2 - 16]])
        s = lax.dot_general(tied(kk, ties, C), wq, NTDIMS, preferred_element_type=f32)
        sb = sbs[g % 2]
        if qo == 1:
            mrg = jnp.where(C["tri"], s[n - 32:n], s[n - 64:n - 32])
            mid = s[0:n - 64]
        elif qo == 2:
            mrg = jnp.where(C["tri"], s[32:64], s[0:32])
            mid = s[64:n]
        elif kmin == 0:
            mrg = jnp.where(C["tri"], s[n - 32:n], s[0:32])
            mid = s[32:n - 32]
        else:
            mrg = jnp.where(C["tri"], s[n - 32:n], -1e30)
            mid = s[0:n - 32]
        m = jnp.max(mrg, axis=0, keepdims=True)
        if mid.shape[0]:
            sb[r + C['za'], 224 - mid.shape[0]:224, :] = mid
            m = jnp.maximum(jnp.max(mid, axis=0, keepdims=True), m)
        sb[r + C['za'], 224:256, :] = mrg
        return s, m

    def softmax_pieces(Q, g, ms, C):
        zero8 = C["zero16"][0:8]
        sb, tb = sbs[g % 2], tbs[g % 2]
        pw = {}

        mg = {}

        def chunk(r, k, hf):
            o = 32 * k + 16 * hf
            src = sb.at[r + C['zb']]
            if r not in mg:
                mg[r] = ms[r] if mg["rel"] is None else jnp.where(C["never"], mg["rel"], ms[r])
            a = jnp.exp2(src[pl.ds(o, 8, stride=2), :] - mg[r])
            b = jnp.exp2(src[pl.ds(o + 1, 8, stride=2), :] - mg[r])
            return _pack2(a, b)

        def col(c, hf):
            hs = slice(8 * hf, 8 * hf + 8)
            X = [None] * 4
            for r in range(4):
                k = c - r
                if k == 0:
                    pw[r, hf] = chunk(r, 7, hf)
                    X[r] = pw[r, hf] & C["mtop"][hs]
                elif k == 8:
                    X[r] = (pw[r, hf] & C["mbot"][hs]) if (r, hf) in pw else chunk(r, 7, hf)
                elif 0 < k < 8:
                    X[r] = chunk(r, k - 1, hf)
            nz = [r for r in range(4) if X[r] is not None]
            if len(nz) == 1:
                r = nz[0]
                T = [jnp.where(C["grp8"] == (j + r) % 4, X[r], zero8) for j in range(4)]
            else:
                def sel(mask, a, b):
                    if a is None and b is None:
                        return None
                    return jnp.where(mask, zero8 if a is None else a, zero8 if b is None else b)
                U = [sel(C["odd"], X[(p + 1) % 4], X[p]) for p in range(4)]
                Tp = [sel(C["hi"], U[(p + 2) % 4], U[p]) for p in range(4)]
                T = [zero8 if Tp[(-j) % 4] is None else Tp[(-j) % 4] for j in range(4)]
            for j in range(4):
                tb[j + C['za'], 16 * c + 8 * hf:16 * c + 8 * hf + 8, :] = T[j]
            return T[0]

        def piece(cs):
            def f(rel):
                mg.clear()
                mg["rel"] = rel
                return functools.reduce(lambda a, b: a | b, [col(c, hf) for c, hf in cs])
            return f
        grps = [[x for x in cs if x[0] >= Q.cmin] for cs in sm_groups(C['SMT'])]
        return [(piece(cs), C['WM']) for cs in grps if cs]

    def pv_j(Q, g, j, C):
        h = 4 * g + j
        off = (DH * h) % 16
        base = DH * h - off
        r1 = (off + DH) % 32
        acc = None
        for t in range(Q.cmin // 4, 3):
            v = vt_ref[Q.at(1, t - 1), base // 2:base // 2 + 16, :]
            halves = [v[0:8], v[8:16]]
            hsel = (r1 // 2) // 8
            halves[hsel] = jnp.where(C["row8"] == (r1 // 2) % 8, jnp.uint32(ONE2), halves[hsel])
            vw = _b(_cat(halves))
            tt = _b(tbs[g % 2][j + C['zb'], 64 * t:64 * t + 64, :])
            d = jnp.dot(vw, tt, preferred_element_type=f32)
            acc = d if acc is None else (d + acc if C['EX'] else acc + d)
        linv = 1.0 / acc[r1:r1 + 1, :]
        lo8 = (off // 8) * 8
        o = acc[lo8:lo8 + 24, :] * linv
        if j:
            o = pltpu.roll(o, 128 - 32 * j, 1)
        ot_ref[DH * h:DH * h + DH, :] = o[off - lo8:off - lo8 + DH, :]
        return _u(o[0:8]) | _u(o[8:16]) | _u(o[16:24])

    def section(stages, load_m, store_m, kn, ks):
        C = attn_consts()
        C.update(kn)
        clock = [0, 0, 0, 0]
        reg = []

        umax = {}

        def place(rows):
            m = clock.index(min(clock))
            s = clock[m]
            clock[m] += rows
            return s

        def token(tm):
            best = None
            for lo, rows, res in reg:
                if lo <= tm and rows:
                    r = min((tm - lo) // 8, rows // 8 - 1)
                    if best is None or lo + 8 * r >= best[0]:
                        best = (lo + 8 * r, res, r)
            return None if best is None else best[1][8 * best[2]:8 * best[2] + 8]

        ms = [m_ref[r, 0:1, :] for r in range(4)] if load_m else None
        last_qk = max(i for i, sp in enumerate(stages) if sp.get("qk"))
        for si, sp in enumerate(stages):
            C.update(kn)
            C.update(ks.get(si, {}))
            for f in sp.get("pre", []):
                f()
            fl = [f for u in sp.get("fl", []) for f in u]
            P = softmax_pieces(sp["sm"][0], sp["sm"][1], ms, C) if sp.get("sm") else []
            B = [pc for a in sp.get("B", []) for pc in battn_pieces(*a, C)]
            X = sp.get("X", [])
            items = [((ip + 1) / len(P), 0, pc) for ip, pc in enumerate(P)]
            bf = C['BF'] if len(B) == 4 else BF2
            if P:
                items += [((int(bf[ib] * len(P)) + 1) / len(P), 1, pc) for ib, pc in enumerate(B)]
                items += [((int(C['XF'] * (ix + 1) / len(X) * len(P)) + 1) / len(P), 2, pc) for ix, pc in enumerate(X)]
            else:
                items += [(bf[ib], 1, pc) for ib, pc in enumerate(B)]
                items += [((ix + 1) / len(X), 2, pc) for ix, pc in enumerate(X)]
            items = sorted(items, key=lambda z: z[:2])
            seq = [z[2] for z in items]
            tbeg = min(clock)
            lead = C['LEAD']
            passes = [("f", u, place(128), 128) for u in range(lead)]
            if sp.get("qk"):
                passes += [("q", r, place(qk_rows(sp["qk"][0], r)), qk_rows(sp["qk"][0], r)) for r in range(4)]
            if sp.get("pv"):
                passes += [("p", j, [place(32) for _ in range(sp["pv"][0].cmin // 4, 3)][0], 0) for j in range(4)]
            nsp = C['LSN'] if si == len(stages) - 1 and C['LSP'] > 1 else 0
            passes += [("f", u, place(128), 128) for u in range(lead, len(fl) - nsp)]
            passes += [("f", u, [place(128 // C['LSP']) for _ in range(C['LSP'])][0], 0) for u in range(len(fl) - nsp, len(fl))]
            tend = min(clock)
            slots = {}
            lastp = 0
            dl = []
            for s, pc in enumerate(seq):
                tm = tbeg + (s + 1) * (tend - tbeg) // len(seq) - C['TO']
                cand = [ip for ip, (kd, _, t0, rows) in enumerate(passes)
                        if ip >= lastp and rows and t0 <= tm < t0 + rows]
                if not cand:
                    cand = [ip for ip, (kd, _, t0, rows) in enumerate(passes)
                            if ip >= lastp and rows and t0 > tm][:1]
                if not cand:
                    cand = [ip for ip, p_ in enumerate(passes) if p_[3]][-1:]
                ip = cand[0]
                lastp = ip
                t0, rows = passes[ip][2], passes[ip][3]
                r8 = min(max(tm - t0, 0) // 16, rows // 16 - 1)
                while any(x[1] == r8 for x in slots.get(ip, [])) and r8 < rows // 16 - 1:
                    r8 += 1
                slots.setdefault(ip, []).append((s, r8))
                dl.append(t0 + 16 * r8)
            ms_n = []
            pvt = []
            for ip, (kd, idx, t0, rows) in enumerate(passes):
                if ip == len(passes) - HOOK:
                    for f in sp.get("hook", []):
                        f()
                ties = []
                for s, r8 in slots.get(ip, []):
                    if seq[s] is None:
                        continue
                    ties.append((r8, seq[s][0](token(dl[s] - seq[s][1]))))
                if kd == "f" and pvt and (t0 >= pvt[0][0] + C['PVD'] or ip == len(passes) - 1):
                    free = [r8 for r8 in range(8) if all(x[0] != r8 for x in ties)]
                    ties.append((free[0], functools.reduce(lambda a, b: a | b, [x[1] for x in pvt])))
                    pvt = []
                if kd == "q":
                    sres, m = qk_r(sp["qk"][0], sp["qk"][1], idx, ties, C)
                    ms_n.append(m)
                    reg.append((t0 + C['PL'], rows, sres))
                    if si == last_qk and store_m:
                        m_ref[idx] = jnp.broadcast_to(m, (8, 128))
                elif kd == "p":
                    pvt.append((t0, pv_j(sp["pv"][0], sp["pv"][1], idx, C)))
                    if idx == 3 and sp["pv"][2] is not None:
                        oa_transpose(*sp["pv"][2:])
                else:
                    C['split'] = C['LSP'] if si == len(stages) - 1 and ip >= len(passes) - C['LSN'] else 1
                    key = (fl[idx].func, id(fl[idx].args[-1]))
                    umax[key] = max(umax.get(key, 0), t0) if C['EX'] else t0
                    reg.append((umax[key] + C['PL'], rows, fl[idx](ties, C)))
            if sp.get("qk"):
                ms = ms_n
            for f in sp.get("post", []):
                f()

    def attn_stages(Q, oa_prev, first=False, last=False):
        sts = []
        for g in range(NG):
            sp = dict(sm=(Q, g), fl=[], B=[], X=[], pre=[], post=[], hook=[])
            if not (last and g == NG - 1):
                sp["qk"] = (Q, g + 1) if g + 1 < NG else (Q + 1, 0)
            if g > 0:
                sp["pv"] = (Q, g - 1, None)
            elif not first:
                sp["pv"] = (Q + (-1), NG - 1, oa_prev)
            sts.append(sp)
        return sts

    def spread(sts, F, cnt):
        assert sum(cnt) == len(F), (sum(cnt), len(F))
        k = 0
        for sp, c in zip(sts, cnt):
            sp["fl"] += F[k:k + c]
            k += c

    def U_qk(Q, ns):
        return [unit(qk_pass, Q, n) for n in ns]

    def U_v(Q):
        return [unit(v_pass, Q, n) for n in range(NT)]

    def U_pb(Q, pn, ns=range(15)):
        return [unit(pb_pass, Q, pn, n) for n in ns]

    def now(pcs):
        return lambda: [pc[0](None) for pc in pcs]

    Z = [Blk(None, b) for b in range(NB)]
    xmb = [[xm_piece(Z[b], i) for i in range(4)] for b in range(4)]
    gps = [g_piece(Z[b], i) for b in range(4) for i in range(4)]

    def U_xw(bs, ns):
        return [u for n in ns for b in bs for u in U_qk(Z[b], [n])]

    rest = U_xw(range(XA, 4), range(WB))
    nsp = WB - 2
    fls = ([U_xw(range(XA), range(WA)), U_xw(range(XA), range(WA, WB))] +
           [rest[len(rest) * i // nsp:len(rest) * (i + 1) // nsp] for i in range(nsp)] +
           [U_xw(range(4), [n]) for n in range(WB, 7)])
    pre = [dict(fl=fl, pre=[], X=gps[16 * (n - 2) // 5:16 * (n - 1) // 5] if n > 1 else []) for n, fl in enumerate(fls)]
    pre[1]["X"] = [p for b in range(XA, 4) for p in xmb[b]]
    pre[0]["pre"] = [c_x.wait, cp_wb(1).start, cp_wb(2).start, now([p for b in range(XA) for p in xmb[b]]), cw[0].wait,
                     c_wv.start]
    pre[1]["pre"] = [c_gw.wait, c_x2.wait, cw[1].wait, c_woa.start, c_wob.start]
    pre[WB]["pre"] = [cw[2].wait, c_xl.start]

    def st(fl, **kw):
        d = dict(fl=fl, pre=[], X=[], B=[])
        d.update(kw)
        return d

    pb = {(b, p): U_pb(Z[b], (2, 1, 0)[b], range(5 * p, 5 * p + 5)) for b in range(3) for p in range(3)}
    pwb = [[prep_wb(p, c) for c in range(NT)] for p in range(3)]
    BB = [(2, obs[0], True, i) for i in range(NG)] + [(1, obs[1], False, i) for i in range(NG)]
    pre.append(st(U_qk(Z[0], WORD[7:10]) + U_qk(Z[1], WORD[7:10]), pre=[cw[3].wait, cp_wb(0).wait],
                  X=[None] + pwb[0][0:2]))
    pre.append(st(U_qk(Z[2], WORD[7:10]) + U_qk(Z[3], WORD[7:10]), X=pwb[0][2:5] + [None]))
    pre.append(st(pb[0, 0]))
    pre.append(st(pb[1, 0][:PB1]))
    pre.append(st(pb[1, 0][PB1:] + pb[2, 0], pre=[cp_wb(1).wait, cp_wb(2).wait], X=[None] * XN + pwb[1]))
    pre.append(st(pb[0, 1], X=pwb[2] + [None]))
    pre.append(st(pb[0, 2] + pb[1, 1][:PB2], pre=[c_wv.wait], X=[None] * XN + [prep_wv(c) for c in range(NT)]))
    v0 = U_v(Z[0])
    ee = [st(v0[0:2], B=[BB[0]]), st(v0[2:5], qk=(Z[0], 0), B=[BB[1]])]
    b0 = attn_stages(Z[0], None, first=True)
    b1 = attn_stages(Z[1], oas[0])
    spread(b0 + b1, pb[1, 1][PB2:] + pb[1, 2] + U_v(Z[1]) + pb[2, 1] + pb[2, 2] + U_v(Z[2]) + U_o(Z[0], oas[0], obs[0]), B01CNT)
    for i, s in enumerate(B1POS):
        (b0 + b1)[s]["B"].append(BB[2 + i])
    (b0 + b1)[B1POS[6]]["pre"].append(lambda: halo_copy(1, 2))
    b0[P7]["pre"] += [c_woa.wait, c_wob.wait]
    for c in range(NT):
        (b0 + b1)[P7 + 1 + c]["X"].append(prep_wob(c))
    pre = pre + ee + b0 + b1
    for s in HB:
        pre[s]["fl"].insert(0, pre[8]["fl"].pop())
    section(pre, False, True, KP, SP)
    c_xl.wait()

    def mid_block(Q, b):
        par, q3 = (2 - Q.off) % 3, Q.off % 3
        sts = attn_stages(Q, oas[0])
        sts[0]["pre"].append(lambda: halo_copy(par, (par + 1) % 3))
        src = dict(b=U_pb(Q + 1, (par + 2) % 3), o=U_o(Q + (-1), oas[0], obs[(q3 + 2) % 3]), v=U_v(Q + 1),
                   q=U_qk(Q + 2, range(5)), k=U_qk(Q + 2, range(5, 10)))
        for sp, w in zip(sts, (ORD, ORD3, ORD2)[b].split()):
            sp["fl"] += [src[ch].pop(0) for ch in w]
        assert not any(src.values())
        for g in range(NG):
            sts[g]["B"] = [(par, obs[q3], False, g)]
        for i in range(4):
            sts[i // 2]["X"].append(xm_piece(Q + 2, i))
            sts[4 + i]["X"].append(g_piece(Q + 2, i))
        return sts

    def p2(i, carry):
        Q = Blk(i, 2)
        section([sp for b in range(BPI) for sp in mid_block(Q + b, b)], True, True, KL, SL)
        return carry

    lax.fori_loop(0, 12 // BPI, p2, 0)
    cp_o(0, 13 * TB, 6).start()

    b14 = attn_stages(Z[14], oas[1])
    b14[0]["pre"].append(lambda: halo_copy(0, 1))
    b15 = attn_stages(Z[15], oas[0], last=True)
    b15[0]["pre"].append(lambda: halo_copy(2, 0))
    src = dict(b=U_pb(Z[15], 2), v=U_v(Z[15]), o=U_o(Z[13], oas[1], obs[1]), p=U_o(Z[14], oas[0], obs[2]))
    for si, (sp, w) in enumerate(zip(b14 + b15, EORD.split())):
        assert all({"b": si < 8, "v": si < 9, "o": si < 15, "p": si > 8}[ch] for ch in w)
        sp["fl"] += [src[ch].pop(0) for ch in w]
        if "o" in w and not src["o"]:
            sp["post"].append(cp_o(13 * TB, TB, 7).start)
    assert not any(src.values())
    for g in range(NG):
        b14[g]["B"] = [(0, obs[2], False, g)]
        b15[g]["B"] = [(2, obs[0], False, g)]
    b15[7]["pv"] = (Z[15], NG - 2, oas[1], range(NT - 1))
    early = []
    for n in range(NT):
        s_ = {}
        early.append([functools.partial(ob_pass, obs[0], n, k, s_) for k in range(NT)] +
                     [functools.partial(oa_early, Z[15], oas[1], n, k, s_) for k in range(NT - 1)])
    late = [[functools.partial(oa_late, Z[15], oas[1], n, h, LS) for h in range(LS) for n in range(NT)]]
    tail = [dict(pre=[cp_o(14 * TB, TB, 8).start], pv=(Z[15], NG - 1, oas[1], [NT - 1]), fl=early + late)]
    section(b14 + b15 + tail, True, False, KE, SE)
    cp_o(0, 13 * TB, 6).wait()
    for k in range(2):
        cp_o((13 + k) * TB, TB, 7 + k).wait()
    for h in range(LS):
        cp_o(15 * TB + TB // LS * h, TB // LS, 9).wait()


@jax.jit
def pallas_gated_mix__sliding_block__sliding_local_dilated__prompt_kernel(A_x, A_wqkv, A_wo, B_x, B_wqkv, B_wo, gate_w):
    x = A_x.reshape(S, D)
    bbuf = [pltpu.VMEM((NT, TB, 128), f32), pltpu.VMEM((NT + 1, 2, HALO + TB // 2, 128), f32),
            pltpu.VMEM((NT + 1, 2, HALO + TB // 2, 128), f32)]
    out = pl.pallas_call(
        kernel,
        out_shape=jax.ShapeDtypeStruct((S, D), bf16),
        in_specs=[pl.BlockSpec(memory_space=pl.ANY)] * 6,
        out_specs=pl.BlockSpec(memory_space=pl.ANY),
        scratch_shapes=[
            pltpu.VMEM((S, D), bf16),
            pltpu.VMEM((D, 2 * D), bf16),
            pltpu.VMEM((D, D), bf16),
            pltpu.VMEM((D, D), bf16),
            pltpu.VMEM((3, D, D), bf16),
            pltpu.VMEM((D, D), bf16),
            pltpu.VMEM((D,), bf16),
            pltpu.VMEM((S, D), bf16),
            pltpu.SemaphoreType.DMA((5,)),
            pltpu.VMEM((3 * NT, D // 2, 128), u32),
            pltpu.VMEM((NT, S // 2, 128), u32),
            pltpu.VMEM((NT, S // 2, 128), u32),
            pltpu.VMEM((S, 128), f32),
            pltpu.VMEM((NT, S // 2, 128), u32),
            pltpu.VMEM((NG, S // 2, 128), u32),
            pltpu.VMEM((NB + 1, D // 2, 128), u32),
            pltpu.VMEM((D // 2, D), u32),
            pltpu.VMEM((3 * D // 2, D), u32),
            pltpu.VMEM((D // 2, D), u32),
            pltpu.VMEM((NT, D // 2, 128), u32),
        ] + bbuf + bbuf + bbuf + [
            pltpu.VMEM((D, 128), f32),
            pltpu.VMEM((1, TB // 2, D), u32),
            pltpu.VMEM((1, TB // 2, D), u32),
            pltpu.VMEM((1, TB // 2, D), u32),
            pltpu.VMEM((1, TB // 2, D), u32),
            pltpu.VMEM((1, TB // 2, D), u32),
            pltpu.VMEM((4, 256, 128), f32),
            pltpu.VMEM((4, 256, 128), f32),
            pltpu.VMEM((4, 192, 128), u32),
            pltpu.VMEM((4, 192, 128), u32),
            pltpu.VMEM((4, 8, 128), f32),
            pltpu.SMEM((3,), jnp.int32),
        ],
        compiler_params=pltpu.CompilerParams(vmem_limit_bytes=100 * 1024 * 1024),
    )(x, A_wqkv, A_wo, B_wqkv, B_wo, gate_w)
    return out.reshape(1, S, D)
```
